```python
import jax
import jax.numpy as jnp

def _softmax(x, axis=-1):
    return jax.nn.softmax(x, axis=axis)
def _gelu(x):
    return jax.nn.gelu(x, approximate=True)
def _silu(x):
    return jax.nn.silu(x)
def _sigmoid(x):
    return jax.nn.sigmoid(x)
def _layernorm(x, axis=-1, eps=1e-5):
    m = jnp.mean(x, axis=axis, keepdims=True)
    v = jnp.var(x, axis=axis, keepdims=True)
    return (x - m) / jnp.sqrt(v + eps)
def _scatter_add(tgt, idx, src, axis=0):
    return tgt.at[idx].add(src)
def _segment_sum(src, seg, n):
    return jax.ops.segment_sum(src, seg, n)
class _Rng:
    def __init__(self, key):
        self._k = key
    def _next(self):
        self._k, sub = jax.random.split(self._k)
        return sub
    def normal(self, shape):
        return jax.random.normal(self._next(), shape, dtype=jnp.bfloat16)
    def randint(self, lo, hi, shape):
        return jax.random.randint(self._next(), shape, lo, hi, dtype=jnp.int32)
    def uniform(self, shape, lo=0.0, hi=1.0):
        return jax.random.uniform(self._next(), shape, jnp.bfloat16, lo, hi)
    def permutation(self, n):
        return jax.random.permutation(self._next(), n)


kernel_name = 'recurrent_scan__sliding_local_dilated__geglu_ffn__prompt'

def setup_inputs():
    _rng = _Rng(jax.random.key(int.from_bytes(__import__("os").urandom(4), "little")))
    _w = (lambda a: (lambda t: t.astype(jnp.bfloat16) if jnp.issubdtype(t.dtype, jnp.floating) else t)(jnp.asarray(a)))
    def _A_setup():
        B, S, D = 1, 2048, 1024
        return {
            "x": _w((lambda *s: _rng.normal(s) * 0.05)(B, S, D)),
            "wqkv": _w((lambda *s: _rng.normal(s) * 0.05)(D, 3 * D)),
            "wo": _w((lambda *s: _rng.normal(s) * 0.05)(D, D)),
        }
    _A_in = _A_setup()

    def _B_setup():
        B, S, D, F = 1, 2048, 1024, 3584
        return {
            "x": _w((lambda *s: _rng.normal(s) * 0.05)(B, S, D)),
            "w_gate": _w((lambda *s: _rng.normal(s) * 0.05)(D, F)),
            "w_up": _w((lambda *s: _rng.normal(s) * 0.05)(D, F)),
            "w_down": _w((lambda *s: _rng.normal(s) * 0.05)(F, D)),
        }
    _B_in = _B_setup()

    return {
        "A_x": _A_in["x"],
        "A_wqkv": _A_in["wqkv"],
        "A_wo": _A_in["wo"],
        "B_x": _B_in["x"],
        "B_w_gate": _B_in["w_gate"],
        "B_w_up": _B_in["w_up"],
        "B_w_down": _B_in["w_down"],
    }

def reference(A_x, A_wqkv, A_wo, B_x, B_w_gate, B_w_up, B_w_down):
    def _A_ref(x, wqkv, wo):
        B, S, D = x.shape
        H = 32; Dh = D // H
        W, dil = 8, 2
        qkv = (lambda x, *d: x.transpose(*d))((x @ wqkv).reshape(B, S, 3, H, Dh), 2, 0, 3, 1, 4)
        q, k, v = qkv[0], qkv[1], qkv[2]
        scale = Dh ** -0.5
        pos = jnp.arange(S)
        off = jnp.arange(W) * dil
        idx = pos[:, None] - off[None, :]
        mask = idx >= 0
        idx_c = jnp.where(mask, idx, 0).reshape(-1)
        kg = k[:, :, idx_c, :].reshape(B, H, S, W, Dh)
        vg = v[:, :, idx_c, :].reshape(B, H, S, W, Dh)
        logits = jnp.einsum("bhsd,bhswd->bhsw", q, kg) * scale
        logits = jnp.where(mask[None, None, :, :], logits, -1e9)
        attn = _softmax(logits, axis=-1)
        o = jnp.einsum("bhsw,bhswd->bhsd", attn, vg)
        return (lambda x, *d: x.transpose(*d))(o, 0, 2, 1, 3).reshape(B, S, D) @ wo

    def _B_ref(x, w_gate, w_up, w_down):
        return (_gelu(x @ w_gate) * (x @ w_up)) @ w_down

    x = A_x
    xn = _layernorm(x, axis=-1)
    s = _A_ref(xn, A_wqkv, A_wo)
    g = _silu(_B_ref(xn, B_w_gate, B_w_up, B_w_down))
    return x + s * g
```

```python
import functools
import jax
import jax.numpy as jnp
import numpy as np
import jax.experimental.pallas as pl
import jax.experimental.pallas.tpu as pltpu

S, D, F = 2048, 1024, 3584
H, DH, W, DIL = 32, 32, 8, 2
HALO = 16

def _gelu(x):
    c = 0.7978845608028654
    return 0.5 * x * (1.0 + jnp.tanh(c * (x + 0.044715 * (x * x * x))))

def build(TM=256, FC=512):
    def kern(x_ref, wqkv_ref, wo_ref, wg_ref, wu_ref, wd_ref, o_ref, k_sc, v_sc):
        i = pl.program_id(0)
        @pl.when(i == 0)
        def _():
            k_sc[pl.ds(0, HALO), :] = jnp.zeros((HALO, D), jnp.float32)
            v_sc[pl.ds(0, HALO), :] = jnp.zeros((HALO, D), jnp.float32)
        @pl.when(i > 0)
        def _():
            k_sc[pl.ds(0, HALO), :] = k_sc[pl.ds(TM, HALO), :]
            v_sc[pl.ds(0, HALO), :] = v_sc[pl.ds(TM, HALO), :]
        x = x_ref[...].astype(jnp.float32)
        m = jnp.mean(x, axis=-1, keepdims=True)
        xc = x - m
        var = jnp.mean(xc * xc, axis=-1, keepdims=True)
        xn = (xc * jax.lax.rsqrt(var + 1e-5)).astype(jnp.bfloat16)
        q = jnp.dot(xn, wqkv_ref[:, 0:D], preferred_element_type=jnp.float32) * (DH ** -0.5)
        k_sc[pl.ds(HALO, TM), :] = jnp.dot(xn, wqkv_ref[:, D:2*D], preferred_element_type=jnp.float32)
        v_sc[pl.ds(HALO, TM), :] = jnp.dot(xn, wqkv_ref[:, 2*D:3*D], preferred_element_type=jnp.float32)
        r = jax.lax.broadcasted_iota(jnp.int32, (128, 128), 0) // DH
        c = jax.lax.broadcasted_iota(jnp.int32, (128, 128), 1) // DH
        E = (r == c).astype(jnp.bfloat16)
        pos = i * TM + jax.lax.broadcasted_iota(jnp.int32, (TM, 128), 0)
        outs = []
        for g in range(D // 128):
            sl = slice(g * 128, (g + 1) * 128)
            qg = q[:, sl]
            ls = []
            for w in range(W):
                kw = k_sc[pl.ds(HALO - DIL * w, TM), sl]
                l = jnp.dot((qg * kw).astype(jnp.bfloat16), E, preferred_element_type=jnp.float32)
                if w > 0:
                    l = jnp.where(pos >= DIL * w, l, -1e9)
                ls.append(l)
            mx = functools.reduce(jnp.maximum, ls)
            ps = [jnp.exp(l - mx) for l in ls]
            den = functools.reduce(jnp.add, ps)
            acc = None
            for w in range(W):
                t = ps[w] * v_sc[pl.ds(HALO - DIL * w, TM), sl]
                acc = t if acc is None else acc + t
            outs.append((acc / den).astype(jnp.bfloat16))
        o = jnp.concatenate(outs, axis=1)
        s = jnp.dot(o, wo_ref[...], preferred_element_type=jnp.float32)
        y = None
        for f in range(F // FC):
            fs = slice(f * FC, (f + 1) * FC)
            gt = jnp.dot(xn, wg_ref[:, fs], preferred_element_type=jnp.float32)
            up = jnp.dot(xn, wu_ref[:, fs], preferred_element_type=jnp.float32)
            h = (_gelu(gt) * up).astype(jnp.bfloat16)
            t = jnp.dot(h, wd_ref[fs, :], preferred_element_type=jnp.float32)
            y = t if y is None else y + t
        gsil = y * jax.nn.sigmoid(y)
        o_ref[...] = (x + s * gsil).astype(o_ref.dtype)

    def fn(A_x, A_wqkv, A_wo, B_x, B_w_gate, B_w_up, B_w_down):
        x = A_x.reshape(S, D)
        full = lambda a: pl.BlockSpec(a.shape, lambda i: (0, 0), pipeline_mode=pl.Buffered(1))
        out = pl.pallas_call(
            kern,
            grid=(S // TM,),
            in_specs=[pl.BlockSpec((TM, D), lambda i: (i, 0)), full(A_wqkv), full(A_wo), full(B_w_gate), full(B_w_up), full(B_w_down)],
            out_specs=pl.BlockSpec((TM, D), lambda i: (i, 0)),
            out_shape=jax.ShapeDtypeStruct((S, D), A_x.dtype),
            scratch_shapes=[pltpu.VMEM((TM + HALO, D), jnp.float32), pltpu.VMEM((TM + HALO, D), jnp.float32)],
            compiler_params=pltpu.CompilerParams(dimension_semantics=("arbitrary",), vmem_limit_bytes=110 * 1024 * 1024),
        )(x, A_wqkv, A_wo, B_w_gate, B_w_up, B_w_down)
        return out.reshape(A_x.shape)
    return fn

pallas_recurrent_scan__sliding_local_dilated__geglu_ffn__prompt_kernel = jax.jit(build())
```

```python
import functools

import jax
import jax.numpy as jnp
import jax.experimental.pallas as pl
import jax.experimental.pallas.tpu as pltpu

S, D, F = 2048, 1024, 3584
DH, W, DIL = 32, 8, 2
HALO = 16
L = 128
TM = 256
QR = TM // 4
NT = S // TM
QK = D // 4
NCH = F // (4 * L)
f32, bf16, u32 = jnp.float32, jnp.bfloat16, jnp.uint32
LOG2E = 1.4426950408889634

A_TERMS = ((0, 1, 3), (2, 1, 3), (0,), (3,), (0, 1, 1), (2, -1, 0), (1, -1, 3))
B_TERMS = ((0, 1, 3), (0,), (1, -1, 3), (2, -1, 0), (3,), (0, 1, 1), (2, 1, 3))
ORDER = (1, 3, 2, 4, 0, 6, 5)


def lin(term, get):
    if len(term) == 1:
        return get(term[0])
    a, b = get(term[0]), get(term[2])
    return a + b if term[1] > 0 else a - b


def combine(st, p, m):
    if p == 1:
        st["t"] = m
    elif p == 3:
        st["a"] = m
        return 2, st["t"] + m
    elif p == 2:
        st["d"] = m - st["t"]
        st["t"] = m
    elif p == 4:
        st["a"] = st["a"] - m
        return 1, st["t"] + m
    elif p == 0:
        st["a"] = st["a"] + m
        st["d"] = st["d"] + m
    elif p == 6:
        return 0, st["a"] + m
    else:
        return 3, st["d"] + m
    return None


def outer_blocks(terms, p, get):
    return [lin(terms[p], lambda o: get(2 * (o // 2) + s // 2, 2 * (o % 2) + s % 2)) for s in range(4)]


def cat(xs, axis):
    return xs[0] if len(xs) == 1 else jnp.concatenate(xs, axis)


def mxu(a, b):
    return jnp.dot(pltpu.bitcast(a, bf16), pltpu.bitcast(b, bf16), preferred_element_type=f32)


class Side:
    def __init__(self, jobs, ticks):
        self.jobs, self.ticks, self.n, self.done = list(jobs), ticks, 0, 0

    def __call__(self):
        self.n += 1
        while self.done < len(self.jobs) and self.done * self.ticks < self.n * len(self.jobs):
            self.jobs[self.done]()
            self.done += 1

    def flush(self):
        self.n = self.ticks
        self()


def inner_product(deep, lhs, rhs, emit, side):
    if deep:
        st = {}
        for q in ORDER:
            r = combine(st, q, mxu(lhs(q), rhs(q)))
            if r is not None:
                emit(*r)
            side()
    else:
        a = cat([cat([lhs(0), lhs(1)], 1), cat([lhs(2), lhs(3)], 1)], 0)
        for j in range(2):
            c = mxu(a, cat([rhs(j), rhs(2 + j)], 0))
            n = c.shape[0] // 2
            emit(j, c[:n])
            emit(2 + j, c[n:])
            side()


def outer_emit(states, key, p, sink):
    def emit(s, m):
        r = combine(states.setdefault((key, s), {}), p, m)
        if r is not None:
            o, val = r
            sink(2 * (o // 2) + s // 2, 2 * (o % 2) + s % 2, val)
    return emit


def geglu2(g, u):
    c = 0.7978845608028654
    th = jnp.tanh(g * (g * g * (c * 0.044715) + c))
    a = g * u
    return a * th + a


def interleave_heads(cols):
    cols = list(cols)
    lane = jax.lax.broadcasted_iota(jnp.int32, cols[0].shape, 1)
    for b in range(3):
        s = 4 << b
        m = (lane & s) != 0
        for g in range(8):
            if not g & (1 << b):
                h = g | (1 << b)
                lo, hi = cols[g], cols[h]
                cols[g] = jnp.where(m, pltpu.roll(hi, s, 1), lo)
                cols[h] = jnp.where(m, hi, pltpu.roll(lo, L - s, 1))
    idx = (lane & 0x1C) | ((lane & 3) << 5) | (lane >> 5)
    return [jnp.take_along_axis(c, idx, axis=1) for c in cols]


def transpose8(vs):
    vs = list(vs)
    sub = jax.lax.broadcasted_iota(jnp.int32, vs[0].shape, 0)
    for b in range(3):
        s = 1 << b
        m = (sub & s) != 0
        for g in range(8):
            if not g & s:
                lo, hi = vs[g], vs[g | s]
                vs[g] = jnp.where(m, pltpu.roll(hi, s, 0), lo)
                vs[g | s] = jnp.where(m, hi, pltpu.roll(lo, 8 - s, 0))
    return vs


def build(DQK=0, DV=0, DO=0, RT=128, RT0=64, SLAB=48, SCOPES=0):
    deep_t = (DQK, DQK, DV)
    nq = lambda deep: 7 if deep else 4
    NXA = 7 if all(deep_t) else 9
    PLAIN = (2, 7, 8, 3)

    def inner_ops(terms, deep, blk):
        return [lin(t, lambda s: blk[s]) for t in terms] if deep else blk

    def kern(x_hbm, wqkv_hbm, wo_hbm, wg_hbm, wu_hbm, wd_hbm, out_hbm,
             x_v, xa, h_v, tgu, td, tq, tk, tv, to,
             raw_gu, raw_d, raw_d6, raw_qkv, raw_o,
             ha, oa, q_sc, k_sc, v_sc, obuf,
             x_sem, gu0_sem, gu_sem, side_sem, d6_sem, out_sem):
        xa32, tgu32, td32, to32, ha32, oa32 = (r.bitcast(u32) for r in (xa, tgu, td, to, ha, oa))
        tqkv = (tq, tk, tv)

        def x_copy(r):
            return pltpu.make_async_copy(x_hbm.at[pl.ds(r * TM, TM)], x_v.at[pl.ds(r * TM, TM)], x_sem.at[r])

        def gu0_copies(o):
            rows, cols = pl.ds((o // 2) * 2 * QK, 2 * QK), pl.ds((o % 2) * 2 * L, 2 * L)
            return [pltpu.make_async_copy(w.at[rows, cols], raw_gu.at[0, t, rows, cols], gu0_sem.at[o])
                    for t, w in enumerate((wg_hbm, wu_hbm))]

        def gu_copies(c):
            slot = c % 3
            cols = pl.ds(pl.multiple_of(c * 4 * L, 4 * L), 4 * L)
            return [pltpu.make_async_copy(w.at[:, cols], raw_gu.at[slot, t], gu_sem.at[slot])
                    for t, w in enumerate((wg_hbm, wu_hbm))]

        def slab_row(it):
            return pl.multiple_of(jnp.minimum(it * SLAB, QK - SLAB), 16)

        def side_copies(it):
            slot = it % 2
            sem = side_sem.at[slot]
            cps = [pltpu.make_async_copy(wd_hbm.at[pl.ds(pl.multiple_of(it * 4 * L, 4 * L), 4 * L)], raw_d.at[slot], sem)]
            r0 = slab_row(it)
            for i in range(4):
                cps.append(pltpu.make_async_copy(wqkv_hbm.at[pl.ds(i * QK + r0, SLAB)], raw_qkv.at[slot, i], sem))
            u = jnp.minimum(it, 3)
            rows = pl.ds(pl.multiple_of((u // 2) * 512, 512), 512)
            for j in range(4):
                cols = pl.ds(pl.multiple_of((2 * j + u % 2) * L, L), L)
                cps.append(pltpu.make_async_copy(wo_hbm.at[rows, cols], raw_o.at[slot, j], sem))
            return cps

        d6_copy = pltpu.make_async_copy(wd_hbm.at[pl.ds((NCH - 1) * 4 * L, 4 * L)], raw_d6, d6_sem.at[0])

        def start(cps):
            for cp in cps:
                cp.start()

        def wait(cps):
            for cp in cps:
                cp.wait()

        x_copy(0).start()
        for o in (0, 2, 1, 3):
            start(gu0_copies(o))
        for r in range(1, NT):
            x_copy(r).start()
        start(gu_copies(1))
        start(gu_copies(2))
        start(side_copies(0))
        d6_copy.start()

        def ln_job(r, u):
            def norm(i):
                x = x_v[pl.ds(r * TM + i * QR + u * 16, 16), :].astype(f32)
                xc = x - jnp.mean(x, axis=-1, keepdims=True)
                var = jnp.mean(xc * xc, axis=-1, keepdims=True)
                return xc * jax.lax.rsqrt(var + 1e-5)
            xn = [norm(i) for i in range(4)]
            for cg in range(2):
                for p in ORDER:
                    blk = outer_blocks(A_TERMS, p, lambda i, j: xn[i][:, (2 * j + cg) * L:(2 * j + cg + 1) * L])
                    ops = inner_ops(A_TERMS, True, blk) + [blk[1], blk[2]]
                    for q in range(NXA):
                        xa[p, q, cg, pl.ds(r * QR + u * 16, 16), :] = ops[q].astype(bf16)

        def gu_job(slot, p, t, u):
            blk = outer_blocks(B_TERMS, p, lambda i, j: raw_gu[slot, t, pl.ds(i * QK + u * 16, 16), pl.ds(j * L, L)].astype(f32))
            for q, v in enumerate(inner_ops(B_TERMS, True, blk)):
                tgu[p, q, t, pl.ds(u * 16, 16), :] = v.astype(bf16)

        def gu_jobs(slot, p):
            return [functools.partial(gu_job, slot, p, t, u) for u in range(QK // 16) for t in range(2)]

        def wd_job(src, r_src, r_dst, cg):
            get = lambda i, j: src[pl.ds(i * L + r_src, 16), pl.ds((2 * j + cg) * L, L)].astype(f32)
            for p in range(7):
                for q, v in enumerate(inner_ops(B_TERMS, True, outer_blocks(B_TERMS, p, get))):
                    td[p, q, cg, pl.ds(r_dst, 16), :] = v.astype(bf16)

        def qkv_job(slot, r0, t, u):
            rows = []
            for i in range(4):
                cols = [pltpu.bitcast(raw_qkv[slot, i, pl.ds(u * 16, 16), pl.ds(t * D + g * L, L)], u32) for g in range(8)]
                rows.append([pltpu.bitcast(c, bf16) for c in interleave_heads(cols)])
            for cg in range(2):
                for p in range(7):
                    blk = outer_blocks(B_TERMS, p, lambda i, j: rows[i][2 * j + cg].astype(f32))
                    for q, v in enumerate(inner_ops(B_TERMS, deep_t[t], blk)):
                        tqkv[t][p, q, cg, pl.ds(r0 + u * 16, 16), :] = v.astype(bf16)

        def wo_jobs(slot, unit):
            new = {}

            def permute(ih, j):
                old = [[raw_o[slot, j, pl.ds(g1 * 256 + s * 32 + ih * 16, 16), :].astype(f32) for s in range(8)] for g1 in range(2)]
                for il in range(2):
                    tr = [transpose8([v[il * 8:(il + 1) * 8] for v in old[g1]]) for g1 in range(2)]
                    for a in range(8):
                        new[2 * ih + il, j, a] = cat([tr[0][a], tr[1][a]], 0)

            def emit(a):
                rows = pl.ds(pl.multiple_of(a * 32 + (unit // 2) * 16, 16), 16)
                for p in range(7):
                    blk = outer_blocks(B_TERMS, p, lambda i, j: new[i, j, a])
                    for q, v in enumerate(inner_ops(B_TERMS, DO, blk)):
                        to[p, q, unit % 2, rows, :] = v.astype(bf16)

            return ([functools.partial(permute, ih, j) for ih in range(2) for j in range(4)]
                    + [functools.partial(emit, a) for a in range(8)])

        def gu_product(c, states, p, r0, rt, side):
            rows = pl.ds(r0 // 2, rt // 2)

            def sink(i, j, gu):
                hh = geglu2(gu[:, :L], gu[:, L:]).astype(bf16)
                for b in range(rt // QR):
                    h_v[c, j, pl.ds((r0 // QR + b) * TM + i * QR, QR), :] = hh[b * QR:(b + 1) * QR]

            inner_product(True,
                          lambda q: cat([xa32[p, q, cg, rows, :] for cg in range(2)], 1),
                          lambda q: cat([tgu32[p, q, t] for t in range(2)], 1),
                          outer_emit(states, r0, p, sink), side)

        tiles0 = RT0 // QR
        for r in range(tiles0):
            x_copy(r).wait()
            for u in range(QR // 16):
                ln_job(r, u)
        wait(gu0_copies(0))
        for job in gu_jobs(0, ORDER[0]):
            job()
        need = {1: (2,), 2: (1, 3)}
        for b in range(NT // tiles0):
            states = {}
            nxt = range((b + 1) * tiles0, min((b + 2) * tiles0, NT))
            ln = None
            for n, p in enumerate(ORDER):
                jobs = []
                if b == 0 and n < 6:
                    for o in need.get(n + 1, ()):
                        wait(gu0_copies(o))
                    jobs = gu_jobs(0, ORDER[n + 1])
                if b == NT // tiles0 - 1 and n == 6:
                    wait(gu_copies(1))
                    jobs = gu_jobs(1, ORDER[0])
                if ln is None and (b > 0 or n == 3):
                    for r in nxt:
                        x_copy(r).wait()
                    ln = Side([functools.partial(ln_job, r, u) for r in nxt for u in range(QR // 16)], 7 * (7 - n))
                side = Side(jobs, 7)

                def both(side=side, ln=ln):
                    side()
                    if ln is not None:
                        ln()
                gu_product(0, states, p, b * RT0, RT0, both)

        def chunk(c, _):
            it = c - 1
            slot = it % 2

            @pl.when(c + 1 < NCH)
            def _():
                wait(gu_copies(c + 1))
                start(side_copies(it + 1))

            @pl.when(c + 2 < NCH)
            def _():
                start(gu_copies(c + 2))

            @pl.when(c == 1)
            def _():
                d6_copy.wait()

            wait(side_copies(it))
            r0 = slab_row(it)
            jobs = [functools.partial(wd_job, raw_d.at[slot], u * 16, pl.multiple_of(it * L + u * 16, 16), cg)
                    for u in range(L // 16) for cg in range(2)]
            r6 = pl.multiple_of(jnp.minimum(it * 32, L - 32), 16)
            jobs += [functools.partial(wd_job, raw_d6, r6 + u * 16, (NCH - 1) * L + r6 + u * 16, cg)
                     for u in range(2) for cg in range(2)]
            jobs += [functools.partial(qkv_job, slot, r0, t, u) for t in range(3) for u in range(SLAB // 16)]
            jobs += wo_jobs(slot, jnp.minimum(it, 3))
            nrt = S // 4 // RT
            extra = Side(jobs, 7 * 7 * nrt)
            states = {}
            for n, p in enumerate(ORDER):
                if n < 6:
                    side = Side(gu_jobs(c % 3, ORDER[n + 1]), 7 * nrt - 2)
                else:
                    side = Side(gu_jobs(jnp.minimum(c + 1, NCH - 1) % 3, ORDER[0]), 7 * nrt - 2)

                def both(side=side):
                    side()
                    extra()
                for b in range(nrt):
                    gu_product(c, states, p, b * RT, RT, both)
            return 0

        jax.lax.fori_loop(1, NCH, chunk, 0)

        def out_copy(r):
            return pltpu.make_async_copy(obuf.at[r % 2], out_hbm.at[pl.ds(pl.multiple_of(r * TM, TM), TM)], out_sem.at[r % 2])

        for g in range(8):
            k_sc[g, pl.ds(TM, HALO), :] = jnp.zeros((HALO, L), f32)
            v_sc[g, pl.ds(TM, HALO), :] = jnp.zeros((HALO, L), f32)

        def matmul(deep, lhs, rhs, sink, side):
            states = {}
            for p in ORDER:
                inner_product(deep, functools.partial(lhs, p), functools.partial(rhs, p),
                              outer_emit(states, 0, p, sink), side)

        def tile(r, _):
            @pl.when(r >= 2)
            def _():
                out_copy(r - 2).wait()

            base = pl.multiple_of(r * TM, TM)
            for g in range(8):
                k_sc[g, pl.ds(0, HALO), :] = k_sc[g, pl.ds(TM, HALO), :]
                v_sc[g, pl.ds(0, HALO), :] = v_sc[g, pl.ds(TM, HALO), :]

            def h_job(c, u):
                get = lambda i, j: h_v[c, j, pl.ds(base + i * QR + u * 16, 16), :].astype(f32)
                for p in ORDER:
                    for q, v in enumerate(inner_ops(A_TERMS, True, outer_blocks(A_TERMS, p, get))):
                        ha[p, q, c, pl.ds(u * 16, 16), :] = v.astype(bf16)

            ticks = lambda deep: 49 if deep else 14
            side = Side([functools.partial(h_job, c, u) for c in range(NCH) for u in range(QR // 16)],
                        sum(ticks(d) for d in deep_t) - 2)
            xrows = pl.ds(pl.multiple_of(r * (QR // 2), QR // 2), QR // 2)
            for t, dst, off in ((1, k_sc, HALO), (0, q_sc, 0), (2, v_sc, HALO)):
                def sink(i, j, val, t=t, dst=dst, off=off):
                    if t == 0:
                        val = val * (DH ** -0.5 * LOG2E)
                    for cg in range(2):
                        dst[2 * j + cg, pl.ds(off + i * QR, QR), :] = val[:, cg * L:(cg + 1) * L]
                        if t == 2 and i == 0:
                            halo = dst[2 * j + cg, pl.ds(0, HALO), :]
                            first = jnp.broadcast_to(val[0:1, cg * L:(cg + 1) * L], (HALO, L))
                            dst[2 * j + cg, pl.ds(0, HALO), :] = jnp.where(r == 0, first, halo)
                t32 = tqkv[t].bitcast(u32)
                deep = deep_t[t]
                matmul(deep,
                       lambda p, q: cat([xa32[p, q if deep else PLAIN[q], cg, xrows, :] for cg in range(2)], 1),
                       lambda p, q: cat([t32[p, q, cg] for cg in range(2)], 1), sink, side)
            side.flush()

            att = {}

            def attn_job(i, u):
                r0 = i * QR + u * 16
                qs = [q_sc[g, pl.ds(r0, 16), :] for g in range(8)]
                ls = []
                for w in range(W):
                    l = functools.reduce(jnp.add, [qs[g] * k_sc[g, pl.ds(r0 + HALO - DIL * w, 16), :] for g in range(8)])
                    l = l + pltpu.roll(l, 64, 1)
                    l = l + pltpu.roll(l, 32, 1)
                    if r0 < HALO and w > 0:
                        pos = base + r0 + jax.lax.broadcasted_iota(jnp.int32, (16, L), 0)
                        l = jnp.where(pos >= DIL * w, l, -1e9 * LOG2E)
                    ls.append(l)
                mx = functools.reduce(jnp.maximum, ls)
                ps = [jnp.exp2(l - mx) for l in ls]
                inv = 1.0 / functools.reduce(jnp.add, ps)
                att[i, u] = [functools.reduce(jnp.add, [ps[w] * v_sc[g, pl.ds(r0 + HALO - DIL * w, 16), :] for w in range(W)]) * inv
                             for g in range(8)]

            def o_job(u):
                for cg in range(2):
                    for p in ORDER:
                        blk = outer_blocks(A_TERMS, p, lambda i, j: att[i, u][2 * j + cg])
                        for q, v in enumerate(inner_ops(A_TERMS, DO, blk)):
                            oa[p, q, cg, pl.ds(u * 16, 16), :] = v.astype(bf16)

            jobs = []
            for u in range(QR // 16):
                jobs += [functools.partial(attn_job, i, u) for i in range(4)] + [functools.partial(o_job, u)]
            side = Side(jobs, 45)
            gate = {}

            def y_sink(i, j, val):
                y2 = val * 0.25
                gate[i, j] = y2 * jnp.tanh(y2) + y2

            matmul(True,
                   lambda p, q: cat([ha32[p, q, c] for c in range(NCH)], 1),
                   lambda p, q: cat([td32[p, q, cg] for cg in range(2)], 1), y_sink, side)
            side.flush()

            def s_sink(i, j, val):
                cols = pl.ds(j * QK, QK)
                xs = x_v[pl.ds(base + i * QR, QR), cols].astype(f32)
                obuf[r % 2, pl.ds(i * QR, QR), cols] = (xs + val * gate[i, j]).astype(bf16)

            matmul(DO,
                   lambda p, q: cat([oa32[p, q, cg] for cg in range(2)], 1),
                   lambda p, q: cat([to32[p, q, cg] for cg in range(2)], 1), s_sink, lambda: None)
            out_copy(r).start()
            return 0

        jax.lax.fori_loop(0, NT, tile, 0)
        out_copy(NT - 2).wait()
        out_copy(NT - 1).wait()

    def fn(A_x, A_wqkv, A_wo, B_x, B_w_gate, B_w_up, B_w_down):
        any_spec = pl.BlockSpec(memory_space=pl.ANY)
        V = pltpu.VMEM
        dma = pltpu.SemaphoreType.DMA
        out = pl.pallas_call(
            kern,
            in_specs=[any_spec] * 6,
            out_specs=any_spec,
            out_shape=jax.ShapeDtypeStruct((S, D), A_x.dtype),
            scratch_shapes=[
                V((S, D), bf16), V((7, NXA, 2, S // 4, L), bf16), V((NCH, 4, S, L), bf16),
                V((7, 7, 2, QK, L), bf16), V((7, 7, 2, F // 4, L), bf16),
                V((7, nq(DQK), 2, QK, L), bf16), V((7, nq(DQK), 2, QK, L), bf16), V((7, nq(DV), 2, QK, L), bf16),
                V((7, nq(DO), 2, QK, L), bf16),
                V((3, 2, D, 4 * L), bf16), V((2, 4 * L, D), bf16), V((4 * L, D), bf16),
                V((2, 4, SLAB, 3 * D), bf16), V((2, 4, 512, L), bf16),
                V((7, 7, NCH, QR, L), bf16), V((7, nq(DO), 2, QR, L), bf16),
                V((8, TM, L), f32), V((8, TM + HALO, L), f32), V((8, TM + HALO, L), f32), V((2, TM, D), bf16),
                dma((NT,)), dma((4,)), dma((3,)), dma((2,)), dma((1,)), dma((2,)),
            ],
            compiler_params=pltpu.CompilerParams(vmem_limit_bytes=127 * 1024 * 1024),
        )(A_x.reshape(S, D), A_wqkv, A_wo, B_w_gate, B_w_up, B_w_down)
        return out.reshape(A_x.shape)

    return fn


pallas_recurrent_scan__sliding_local_dilated__geglu_ffn__prompt_kernel = jax.jit(build())
```

```python
import functools

import jax
import jax.numpy as jnp
import jax.experimental.pallas as pl
import jax.experimental.pallas.tpu as pltpu

S, D, F = 2048, 1024, 3584
DH, W, DIL = 32, 8, 2
HALO = 16
L = 128
TM = 256
QR = TM // 4
NT = S // TM
QK = D // 4
NCH = F // (4 * L)
PAD = 16
f32, bf16, u32 = jnp.float32, jnp.bfloat16, jnp.uint32
LOG2E = 1.4426950408889634
part = functools.partial

A_TERMS = ((0, 1, 3), (2, 1, 3), (0,), (3,), (0, 1, 1), (2, -1, 0), (1, -1, 3))
B_TERMS = ((0, 1, 3), (0,), (1, -1, 3), (2, -1, 0), (3,), (0, 1, 1), (2, 1, 3))
ORDER = (1, 3, 2, 4, 0, 6, 5)


def lin(term, get):
    if len(term) == 1:
        return get(term[0])
    a, b = get(term[0]), get(term[2])
    return a + b if term[1] > 0 else a - b


def combine(st, p, m):
    if p == 1:
        st["t"] = m
    elif p == 3:
        st["a"] = m
        return 2, st["t"] + m
    elif p == 2:
        st["d"] = m - st["t"]
        st["u"] = m
    elif p == 4:
        st["a2"] = st["a"] - m
        return 1, st["u"] + m
    elif p == 0:
        st["a3"] = st["a2"] + m
        st["d2"] = st["d"] + m
    elif p == 6:
        return 0, st["a3"] + m
    else:
        return 3, st["d2"] + m
    return None


def operands(terms, deep, p, get):
    blk = [lin(terms[p], lambda o: get(2 * (o // 2) + s // 2, 2 * (o % 2) + s % 2)) for s in range(4)]
    if deep == 2:
        return [lin(t, lambda s: blk[s]) for t in terms] + [blk[1], blk[2]]
    return [lin(t, lambda s: blk[s]) for t in terms] if deep else blk


def cat(xs, axis):
    return xs[0] if len(xs) == 1 else jnp.concatenate(xs, axis)


def mxu(a, b):
    return jnp.dot(pltpu.bitcast(a, bf16), pltpu.bitcast(b, bf16), preferred_element_type=f32)


def rows16(r):
    return pl.ds(r if isinstance(r, int) else pl.multiple_of(r, 16), 16)


class Side:
    def __init__(self, jobs, ticks, paced=True):
        self.jobs, self.ticks, self.paced, self.n, self.done = list(jobs), ticks, paced, 0, 0

    def __call__(self, val):
        self.n += 1
        while self.done < len(self.jobs) and self.done * self.ticks < self.n * len(self.jobs):
            pace, job = self.jobs[self.done]
            if pace is not None and self.paced:
                pace(val)
            job()
            self.done += 1


def inner_product(deep, lhs, rhs, emit, side, col_major):
    def ticks(m):
        for b in range(m.shape[1] // L if col_major else 1):
            for r in range(m.shape[0] // 8):
                side(m[r * 8:(r + 1) * 8, b * L:(b + 1) * L])

    if deep:
        st = {}
        for q in ORDER:
            m = mxu(lhs(q), rhs(q))
            r = combine(st, q, m)
            if r is not None:
                emit(*r)
            ticks(m)
    else:
        a = cat([cat([lhs(0), lhs(1)], 1), cat([lhs(2), lhs(3)], 1)], 0)
        for j in range(2):
            c = mxu(a, cat([rhs(j), rhs(2 + j)], 0))
            n = c.shape[0] // 2
            emit(j, c[:n])
            emit(2 + j, c[n:])
            ticks(c)


def outer_emit(states, p, sink):
    def emit(s, m):
        r = combine(states[s], p, m)
        if r is not None:
            o, val = r
            sink(2 * (o // 2) + s // 2, 2 * (o % 2) + s % 2, val)
    return emit


def geglu2(g, u):
    c = 0.7978845608028654
    th = jnp.tanh(g * (g * g * (c * 0.044715) + c))
    a = g * u
    return a * th + a


def interleave_heads(cols):
    cols = list(cols)
    lane = jax.lax.broadcasted_iota(jnp.int32, cols[0].shape, 1)
    for b in range(3):
        s = 4 << b
        m = (lane & s) != 0
        for g in range(8):
            if not g & (1 << b):
                h = g | (1 << b)
                lo, hi = cols[g], cols[h]
                cols[g] = jnp.where(m, pltpu.roll(hi, s, 1), lo)
                cols[h] = jnp.where(m, hi, pltpu.roll(lo, L - s, 1))
    idx = (lane & 0x1C) | ((lane & 3) << 5) | (lane >> 5)
    return [jnp.take_along_axis(c, idx, axis=1) for c in cols]


def transpose8(vs):
    vs = list(vs)
    sub = jax.lax.broadcasted_iota(jnp.int32, vs[0].shape, 0)
    for b in range(3):
        s = 1 << b
        m = (sub & s) != 0
        for g in range(8):
            if not g & s:
                lo, hi = vs[g], vs[g | s]
                vs[g] = jnp.where(m, pltpu.roll(hi, s, 0), lo)
                vs[g | s] = jnp.where(m, hi, pltpu.roll(lo, 8 - s, 0))
    return vs


def build(DQK=0, DV=0, DO=0, RT=128, SLAB=48, HJ=1, AJ=16):
    deep_t = (DQK, DQK, DV)
    nq = lambda deep: 7 if deep else 4
    XDEEP = 1 if all(deep_t) else 2
    PLAIN = (2, 7, 8, 3)

    def kern(zero_ref, x_hbm, wqkv_hbm, wo_hbm, wg_hbm, wu_hbm, wd_hbm, out_hbm,
             x_v, xn, xa, h_v, tgu, td, tq, tk, tv, to,
             raw_gu, raw_d, raw_d6, raw_qkv, mid_qkv, raw_o, mid_o,
             ha, oa, q_sc, k_sc, v_sc, g_sc, obuf,
             x_sem, gu0_sem, gu_sem, side_sem, d6_sem, out_sem):
        xa32, tgu32, td32, to32 = (r.bitcast(u32) for r in (xa, tgu, td, to))
        tqkv = (tq, tk, tv)

        def x_copy(r):
            rows = pl.ds(pl.multiple_of(r * TM, TM), TM)
            return pltpu.make_async_copy(x_hbm.at[rows], x_v.at[rows], x_sem.at[r])

        def gu0_copies(o):
            rows, cols = pl.ds((o // 2) * 2 * QK, 2 * QK), pl.ds((o % 2) * 2 * L, 2 * L)
            return [pltpu.make_async_copy(w.at[rows, cols], raw_gu.at[0, t, rows, cols], gu0_sem.at[o])
                    for t, w in enumerate((wg_hbm, wu_hbm))]

        def gu_copies(c):
            slot = c % 3
            cols = pl.ds(pl.multiple_of(c * 4 * L, 4 * L), 4 * L)
            return [pltpu.make_async_copy(w.at[:, cols], raw_gu.at[slot, t, pl.ds(0, D)], gu_sem.at[slot])
                    for t, w in enumerate((wg_hbm, wu_hbm))]

        def slab_row(it):
            return pl.multiple_of(jnp.minimum(it * SLAB, QK - SLAB), 16)

        def side_copies(it):
            slot = it % 2
            sem = side_sem.at[slot]
            cps = [pltpu.make_async_copy(wd_hbm.at[pl.ds(pl.multiple_of(it * 4 * L, 4 * L), 4 * L)],
                                         raw_d.at[slot, pl.ds(0, 4 * L)], sem)]
            r0 = slab_row(it)
            for i in range(4):
                cps.append(pltpu.make_async_copy(wqkv_hbm.at[pl.ds(i * QK + r0, SLAB)], raw_qkv.at[slot, i, pl.ds(0, SLAB)], sem))
            u = jnp.minimum(it, 3)
            rows = pl.ds(pl.multiple_of((u // 2) * 512, 512), 512)
            for j in range(4):
                cols = pl.ds(pl.multiple_of((2 * j + u % 2) * L, L), L)
                cps.append(pltpu.make_async_copy(wo_hbm.at[rows, cols], raw_o.at[slot, j, pl.ds(0, 512)], sem))
            return cps

        d6_copy = pltpu.make_async_copy(wd_hbm.at[pl.ds((NCH - 1) * 4 * L, 4 * L)], raw_d6.at[pl.ds(0, 4 * L)], d6_sem.at[0])

        def start(cps):
            for cp in cps:
                cp.start()

        def wait(cps):
            for cp in cps:
                cp.wait()

        x_copy(0).start()
        start(gu0_copies(0))
        zero = zero_ref[0]

        def opaque(ref):
            return ref.at[pl.ds(zero, ref.shape[0])]

        def pacer(ref):
            r32 = ref.bitcast(f32)
            idx = (0,) * (len(ref.shape) - 2) + (pl.ds(pl.multiple_of(r32.shape[-2] - 8 + zero, 8), 8), pl.ds(0, L))

            def pace(v):
                r32[idx] = v
            return pace

        def operand_jobs(src, terms, deep, get, put):
            pace = pacer(src)

            def job(p):
                for q, v in enumerate(operands(terms, deep, p, get)):
                    put(p, q, v.astype(bf16))
            return [(pace, part(job, p)) for p in ORDER]

        def ln_jobs(r, dst):
            def norm(u, i):
                x = x_v[rows16(r * TM + i * QR + u * 16), :].astype(f32)
                xc = x - jnp.mean(x, axis=-1, keepdims=True)
                var = jnp.mean(xc * xc, axis=-1, keepdims=True)
                xn[rows16(i * QR + u * 16), :] = xc * jax.lax.rsqrt(var + 1e-5)

            def split(u, cg):
                def put(p, q, v):
                    dst[p, q, cg, rows16(u * 16), :] = v
                return operand_jobs(xn, A_TERMS, XDEEP, lambda i, j: xn[rows16(i * QR + u * 16 + zero), pl.ds((2 * j + cg) * L, L)], put)

            jobs = []
            for u in range(QR // 16):
                for i in range(4):
                    jobs += [(pacer(x_v), part(norm, u, i)), (None, lambda: None), (None, lambda: None)]
            jobs += [(None, lambda: None)] * 8
            for u in range(QR // 16):
                for cg in range(2):
                    jobs += split(u, cg)
            return jobs

        def gu_jobs(slot, p):
            def one(t, u):
                def put(p, q, v):
                    tgu[p, q, t, rows16(u * 16), :] = v
                get = lambda i, j: raw_gu[slot, t, rows16(i * QK + u * 16), pl.ds(j * L, L)].astype(f32)
                return operand_jobs(raw_gu, B_TERMS, True, get, put)[ORDER.index(p)]
            return [one(t, u) for u in range(QK // 16) for t in range(2)]

        def wd_jobs(buf, src, r_src, r_dst, cg):
            def put(p, q, v):
                td[p, q, cg, rows16(r_dst), :] = v
            get = lambda i, j: src[rows16(i * L + r_src), pl.ds((2 * j + cg) * L, L)].astype(f32)
            return operand_jobs(buf, B_TERMS, True, get, put)

        def qkv_permute(slot, t, u, i):
            cols = [pltpu.bitcast(raw_qkv[slot, i, rows16(u * 16), pl.ds(t * D + g * L, L)], u32) for g in range(8)]
            for g, c in enumerate(interleave_heads(cols)):
                mid_qkv.bitcast(u32)[t * 8 + g, pl.ds((i * SLAB + u * 16) // 2, 8), :] = c

        def qkv_jobs(r0, t, u, cg):
            def put(p, q, v):
                tqkv[t][p, q, cg, rows16(r0 + u * 16), :] = v
            get = lambda i, j: opaque(mid_qkv)[t * 8 + 2 * j + cg, rows16(i * SLAB + u * 16), :].astype(f32)
            return operand_jobs(mid_qkv, B_TERMS, deep_t[t], get, put)

        def wo_permute(slot, j, i, g1):
            old = [raw_o[slot, j, rows16(g1 * 256 + s * 32 + (i // 2) * 16), :].astype(f32)[(i % 2) * 8:(i % 2 + 1) * 8] for s in range(8)]
            for a, v in enumerate(transpose8(old)):
                mid_o[j, pl.ds(i * L + a * 16 + g1 * 8, 8), :] = v

        def wo_jobs(unit, a):
            def put(p, q, v):
                to[p, q, unit % 2, rows16(a * 32 + (unit // 2) * 16), :] = v
            return operand_jobs(mid_o, B_TERMS, DO, lambda i, j: opaque(mid_o)[j, rows16(i * L + a * 16), :], put)

        def gu_product(c, states, p, tiles, side):
            def sink(i, j, gu):
                hh = geglu2(gu[:, :L], gu[:, L:]).astype(bf16)
                for b, r in enumerate(tiles):
                    h_v[c, j, pl.ds(pl.multiple_of(r * TM + i * QR, QR), QR), :] = hh[b * QR:(b + 1) * QR]

            inner_product(True,
                          lambda q: cat([cat([xa32[r, p, q, cg] for cg in range(2)], 1) for r in tiles], 0),
                          lambda q: cat([tgu32[p, q, t] for t in range(2)], 1),
                          outer_emit(states, p, sink), side, False)

        new_states = lambda: [{} for _ in range(4)]

        x_copy(0).wait()
        for o in (2, 1, 3):
            start(gu0_copies(o))
        x_copy(1).start()
        for _, job in ln_jobs(0, xa.at[0]):
            job()
        wait(gu0_copies(0))
        for r in range(2, NT):
            x_copy(r).start()
        for _, job in gu_jobs(0, ORDER[0]):
            job()
        need = {0: (2,), 1: (1, 3)}
        states = new_states()
        ln = None
        for n, p in enumerate(ORDER):
            for o in need.get(n, ()):
                wait(gu0_copies(o))
            if n == 2:
                x_copy(1).wait()
                start(gu_copies(1))
                start(gu_copies(2))
                start(side_copies(0))
                d6_copy.start()
                ln = Side(ln_jobs(1, xa.at[1]), 56 * (7 - n), False)
            side = Side(gu_jobs(0, ORDER[n + 1]) if n < 6 else [], 40, False)

            def both(v, side=side, ln=ln):
                side(v)
                if ln is not None:
                    ln(v)
            gu_product(0, states, p, [0], both)

        def chunk0_tile(r, _):
            @pl.when(r + 1 < NT)
            def _():
                x_copy(r + 1).wait()

            ln = Side(ln_jobs(jnp.minimum(r + 1, NT - 1), xa.at[r + 1]), 49 * 8 - 8)
            states = new_states()
            for p in ORDER:
                gu_product(0, states, p, [r], ln)
            return 0

        jax.lax.fori_loop(1, NT, chunk0_tile, 0)
        wait(gu_copies(1))
        for _, job in gu_jobs(1, ORDER[0]):
            job()

        def chunk(c, _):
            it = c - 1
            slot = it % 2

            @pl.when(c + 1 < NCH)
            def _():
                wait(gu_copies(c + 1))
                start(side_copies(it + 1))

            @pl.when(c + 2 < NCH)
            def _():
                start(gu_copies(c + 2))

            @pl.when(c == 1)
            def _():
                d6_copy.wait()

            wait(side_copies(it))
            r0 = slab_row(it)
            r6 = pl.multiple_of(jnp.minimum(it * 32, L - 32), 16)
            jobs = []
            for cg in range(2):
                for u in range(L // 16):
                    jobs += wd_jobs(raw_d, raw_d.at[slot], u * 16, it * L + u * 16, cg)
                for u in range(2):
                    jobs += wd_jobs(raw_d6, raw_d6, r6 + u * 16, (NCH - 1) * L + r6 + u * 16, cg)
            perm = [(pacer(raw_qkv), part(qkv_permute, slot, t, u, i)) for t in range(3) for u in range(SLAB // 16) for i in range(4)]
            for n, job in enumerate(perm):
                jobs.insert(n * 4, job)
            jobs += [(pacer(raw_o), part(wo_permute, slot, j, i, g1)) for j in range(4) for i in range(4) for g1 in range(2)]
            for t in range(3):
                for u in range(SLAB // 16):
                    for cg in range(2):
                        jobs += qkv_jobs(r0, t, u, cg)
            for a in range(8):
                jobs += wo_jobs(jnp.minimum(it, 3), a)
            nb = RT // QR
            nrt = NT // nb
            per_p = 7 * S // 4 // 8
            extra = Side(jobs, 7 * per_p - 32)
            states = [new_states() for _ in range(nrt)]
            for n, p in enumerate(ORDER):
                nxt = (c % 3, ORDER[n + 1]) if n < 6 else (jnp.minimum(c + 1, NCH - 1) % 3, ORDER[0])
                side = Side(gu_jobs(*nxt), per_p - 48)

                def both(v, side=side):
                    side(v)
                    extra(v)
                for b in range(nrt):
                    gu_product(c, states[b], p, range(b * nb, (b + 1) * nb), both)
            return 0

        jax.lax.fori_loop(1, NCH, chunk, 0)

        def out_copy(r):
            return pltpu.make_async_copy(obuf.at[r % 2], out_hbm.at[pl.ds(pl.multiple_of(r * TM, TM), TM)], out_sem.at[r % 2])

        for g in range(8):
            k_sc[g, pl.ds(TM, HALO), :] = jnp.zeros((HALO, L), f32)
            v_sc[g, pl.ds(TM, HALO), :] = jnp.zeros((HALO, L), f32)

        def matmul(deep, lhs, rhs, sink, side, col_major):
            states = new_states()
            for p in ORDER:
                inner_product(deep, part(lhs, p), part(rhs, p), outer_emit(states, p, sink), side, col_major)

        def tile(r, _):
            @pl.when(r >= 2)
            def _():
                out_copy(r - 2).wait()

            base = pl.multiple_of(r * TM, TM)
            for g in range(8):
                k_sc[g, pl.ds(0, HALO), :] = k_sc[g, pl.ds(TM, HALO), :]
                v_sc[g, pl.ds(0, HALO), :] = v_sc[g, pl.ds(TM, HALO), :]

            def h_jobs(c, u):
                def put(p, q, v):
                    ha[p, q, c, rows16(u * 16), :] = v
                jobs = operand_jobs(h_v, A_TERMS, True, lambda i, j: h_v[c, j, rows16(base + i * QR + u * 16), :].astype(f32), put)
                if HJ:
                    return jobs
                return [(jobs[0][0], lambda: [job() for _, job in jobs])]

            ticks = lambda deep: 49 * 8 if deep else 14 * 32
            side = Side([j for c in range(NCH) for u in range(QR // 16) for j in h_jobs(c, u)], sum(ticks(d) for d in deep_t) - 40)
            for t, dst, off in ((1, k_sc, HALO), (0, q_sc, 0), (2, v_sc, HALO)):
                def sink(i, j, val, t=t, dst=dst, off=off):
                    if t == 0:
                        val = val * (DH ** -0.5 * LOG2E)
                    for cg in range(2):
                        dst[2 * j + cg, pl.ds(off + i * QR, QR), :] = val[:, cg * L:(cg + 1) * L]
                        if t == 2 and i == 0:
                            halo = dst[2 * j + cg, pl.ds(0, HALO), :]
                            first = jnp.broadcast_to(val[0:1, cg * L:(cg + 1) * L], (HALO, L))
                            dst[2 * j + cg, pl.ds(0, HALO), :] = jnp.where(r == 0, first, halo)
                t32 = tqkv[t].bitcast(u32)
                deep = deep_t[t]
                matmul(deep,
                       lambda p, q: cat([xa32[r, p, q if deep else PLAIN[q], cg] for cg in range(2)], 1),
                       lambda p, q: cat([t32[p, q, cg] for cg in range(2)], 1), sink, side, not deep)

            att = {}
            q_d, k_d, v_d, g_d = (opaque(ref) for ref in (q_sc, k_sc, v_sc, g_sc))

            def logits(r0, ws):
                for w in ws:
                    l = functools.reduce(jnp.add, [q_d[g, pl.ds(r0, AJ), :] * k_d[g, pl.ds(r0 + HALO - DIL * w, AJ), :] for g in range(8)])
                    l = l + pltpu.roll(l, 64, 1)
                    l = l + pltpu.roll(l, 32, 1)
                    if r0 < HALO and w > 0:
                        pos = base + r0 + jax.lax.broadcasted_iota(jnp.int32, (AJ, L), 0)
                        l = jnp.where(pos >= DIL * w, l, -1e9 * LOG2E)
                    att[r0, w] = l

            def softmax(r0):
                ls = [att[r0, w] for w in range(W)]
                mx = functools.reduce(jnp.maximum, ls)
                ps = [jnp.exp2(l - mx) for l in ls]
                inv = 1.0 / functools.reduce(jnp.add, ps)
                att[r0] = [p * inv for p in ps]

            def mix(r0, g):
                v_sc[8 + g, pl.ds(r0, AJ), :] = functools.reduce(
                    jnp.add, [att[r0][w] * v_d[g, pl.ds(r0 + HALO - DIL * w, AJ), :] for w in range(W)])

            def o_jobs(u, cg):
                def put(p, q, v):
                    oa[p, q, cg, rows16(u * 16), :] = v
                return operand_jobs(v_sc, A_TERMS, DO, lambda i, j: v_d[8 + 2 * j + cg, rows16(i * QR + u * 16), :], put)

            starts = list(range(0, TM, AJ))
            jobs = []
            for n in range(len(starts) + 1):
                for w in range(4):
                    if n < len(starts):
                        jobs.append((pacer(k_sc), part(logits, starts[n], (w, w + 4))))
                    if n > 0:
                        jobs += [(pacer(v_sc), part(mix, starts[n - 1], g)) for g in (2 * w, 2 * w + 1)]
                if n < len(starts):
                    jobs.append((None, part(softmax, starts[n])))
            oj = [o_jobs(u, cg) for u in range(QR // 16) for cg in range(2)]
            jobs += [j[n] for n in range(7) for j in oj]
            side = Side(jobs, 49 * 16 - 24)

            def y_sink(i, j, val):
                y2 = val * 0.25
                gt = y2 * jnp.tanh(y2) + y2
                for cg in range(2):
                    g_sc[2 * j + cg, pl.ds(i * QR, QR), :] = gt[:, cg * L:(cg + 1) * L]

            ha32, oa32 = opaque(ha.bitcast(u32)), opaque(oa.bitcast(u32))
            matmul(True,
                   lambda p, q: cat([ha32[p, q, c] for c in range(NCH)], 1),
                   lambda p, q: cat([td32[p, q, cg] for cg in range(2)], 1), y_sink, side, True)

            def s_sink(i, j, val):
                cols = pl.ds(j * QK, QK)
                xs = x_v[pl.ds(base + i * QR, QR), cols].astype(f32)
                gate = cat([g_d[2 * j + cg, pl.ds(i * QR, QR), :] for cg in range(2)], 1)
                obuf[r % 2, pl.ds(i * QR, QR), cols] = (xs + val * gate).astype(bf16)

            matmul(DO,
                   lambda p, q: cat([oa32[p, q, cg] for cg in range(2)], 1),
                   lambda p, q: cat([to32[p, q, cg] for cg in range(2)], 1), s_sink, lambda v: None, False)
            out_copy(r).start()
            return 0

        jax.lax.fori_loop(0, NT, tile, 0)
        out_copy(NT - 2).wait()
        out_copy(NT - 1).wait()

    def fn(A_x, A_wqkv, A_wo, B_x, B_w_gate, B_w_up, B_w_down):
        any_spec = pl.BlockSpec(memory_space=pl.ANY)
        V = pltpu.VMEM
        dma = pltpu.SemaphoreType.DMA
        out = pl.pallas_call(
            kern,
            in_specs=[pl.BlockSpec(memory_space=pltpu.SMEM)] + [any_spec] * 6,
            out_specs=any_spec,
            out_shape=jax.ShapeDtypeStruct((S, D), A_x.dtype),
            scratch_shapes=[
                V((S + PAD, D), bf16), V((TM + PAD, D), f32), V((NT + 1, 7, 5 + 2 * XDEEP, 2, QR, L), bf16),
                V((NCH, 4, S + PAD, L), bf16),
                V((7, 7, 2, QK, L), bf16), V((7, 7, 2, F // 4, L), bf16),
                V((7, nq(DQK), 2, QK, L), bf16), V((7, nq(DQK), 2, QK, L), bf16), V((7, nq(DV), 2, QK, L), bf16),
                V((7, nq(DO), 2, QK, L), bf16),
                V((3, 2, D + PAD, 4 * L), bf16), V((2, 4 * L + PAD, D), bf16), V((4 * L + PAD, D), bf16),
                V((2, 4, SLAB + PAD, 3 * D), bf16), V((24, 4 * SLAB + PAD, L), bf16),
                V((2, 4, 512 + PAD, L), bf16), V((4, 512 + PAD, L), f32),
                V((7, 7, NCH, QR, L), bf16), V((7, nq(DO), 2, QR, L), bf16),
                V((8, TM, L), f32), V((8, TM + HALO + PAD, L), f32), V((16, TM + HALO + PAD, L), f32),
                V((8, TM, L), f32), V((2, TM, D), bf16),
                dma((NT,)), dma((4,)), dma((3,)), dma((2,)), dma((1,)), dma((2,)),
            ],
            compiler_params=pltpu.CompilerParams(vmem_limit_bytes=127 * 1024 * 1024, disable_bounds_checks=True),
        )(jnp.zeros((1,), jnp.int32), A_x.reshape(S, D), A_wqkv, A_wo, B_w_gate, B_w_up, B_w_down)
        return out.reshape(A_x.shape)

    return fn


pallas_recurrent_scan__sliding_local_dilated__geglu_ffn__prompt_kernel = jax.jit(build())
```

```python
import functools

import jax
import jax.numpy as jnp
import jax.experimental.pallas as pl
import jax.experimental.pallas.tpu as pltpu

S, D, F = 2048, 1024, 3584
DH, W, DIL = 32, 8, 2
HALO = 16
L = 128
TM = 256
QR = TM // 4
NT = S // TM
QK = D // 4
NCH = F // (4 * L)
PAD = 16
f32, bf16, u32 = jnp.float32, jnp.bfloat16, jnp.uint32
LOG2E = 1.4426950408889634
part = functools.partial

A_TERMS = ((0, 1, 3), (2, 1, 3), (0,), (3,), (0, 1, 1), (2, -1, 0), (1, -1, 3))
B_TERMS = ((0, 1, 3), (0,), (1, -1, 3), (2, -1, 0), (3,), (0, 1, 1), (2, 1, 3))
ORDER = (1, 3, 4, 0, 6, 2, 5)
FLIP = (0, 1, 0, 0, 1, 1, 1)


def lin(term, get):
    if len(term) == 1:
        return get(term[0])
    a, b = get(term[0]), get(term[2])
    return a + b if term[1] > 0 else a - b


def combine(st, p, m):
    if p == 1:
        st["t"] = m
    elif p == 3:
        st["a"] = m
        return 2, st["t"] + m
    elif p == 4:
        st["a2"] = st["a"] - m
        st["u"] = m
    elif p == 0:
        st["a3"] = st["a2"] + m
        st["d"] = m - st["t"]
    elif p == 6:
        return 0, st["a3"] + m
    elif p == 2:
        st["d2"] = st["d"] + m
        return 1, st["u"] + m
    else:
        return 3, st["d2"] + m
    return None


def operands(terms, deep, p, get):
    flip = FLIP[p] if terms is B_TERMS else 0
    blk = [lin(terms[p], lambda o: get(2 * (o // 2) + s // 2, 2 * (o % 2) + (s % 2 ^ flip))) for s in range(4)]
    if deep == 2:
        return [lin(t, lambda s: blk[s]) for t in terms] + [blk[1], blk[2]]
    return [lin(t, lambda s: blk[s]) for t in terms] if deep else blk


def cat(xs, axis):
    return xs[0] if len(xs) == 1 else jnp.concatenate(xs, axis)


def mxu(a, b):
    return jnp.dot(pltpu.bitcast(a, bf16), pltpu.bitcast(b, bf16), preferred_element_type=f32)


def rows16(r):
    return pl.ds(r if isinstance(r, int) else pl.multiple_of(r, 16), 16)


class Side:
    def __init__(self, jobs, ticks, paced=True):
        self.jobs, self.ticks, self.paced, self.n, self.done = list(jobs), ticks, paced, 0, 0

    def __call__(self, val, weight=1):
        self.n += weight
        while self.done < len(self.jobs) and self.done * self.ticks < self.n * len(self.jobs):
            pace, job = self.jobs[self.done]
            if pace is not None and self.paced:
                pace(val)
            job()
            self.done += 1


def inner_product(deep, lhs, rhs, emit, side, col_major, st):
    def ticks(m):
        for b in range(m.shape[1] // L if col_major else 1):
            for r in range(m.shape[0] // 8):
                side(m[r * 8:(r + 1) * 8, b * L:(b + 1) * L])

    if deep:
        for q in ORDER:
            m = mxu(lhs(q), rhs(q))
            r = combine(st, q, m)
            if r is not None:
                emit(*r)
            ticks(m)
    else:
        a = cat([cat([lhs(0), lhs(1)], 1), cat([lhs(2), lhs(3)], 1)], 0)
        for j in range(2):
            c = mxu(a, cat([rhs(j), rhs(2 + j)], 0))
            n = c.shape[0] // 2
            emit(j, c[:n])
            emit(2 + j, c[n:])
            ticks(c)


def outer_emit(states, p, sink):
    def emit(s, m):
        s ^= FLIP[p]
        r = combine(states[s], p, m)
        if r is not None:
            o, val = r
            sink(2 * (o // 2) + s // 2, 2 * (o % 2) + s % 2, val)
    return emit


def geglu2(g, u):
    c = 0.7978845608028654
    th = jnp.tanh(g * (g * g * (c * 0.044715) + c))
    a = g * u
    return a * th + a


def interleave_heads(cols):
    cols = list(cols)
    lane = jax.lax.broadcasted_iota(jnp.int32, cols[0].shape, 1)
    for b in range(3):
        s = 4 << b
        m = (lane & s) != 0
        for g in range(8):
            if not g & (1 << b):
                h = g | (1 << b)
                lo, hi = cols[g], cols[h]
                cols[g] = jnp.where(m, pltpu.roll(hi, s, 1), lo)
                cols[h] = jnp.where(m, hi, pltpu.roll(lo, L - s, 1))
    idx = (lane & 0x1C) | ((lane & 3) << 5) | (lane >> 5)
    return [jnp.take_along_axis(c, idx, axis=1) for c in cols]


def transpose8(vs):
    vs = list(vs)
    sub = jax.lax.broadcasted_iota(jnp.int32, vs[0].shape, 0)
    for b in range(3):
        s = 1 << b
        m = (sub & s) != 0
        for g in range(8):
            if not g & s:
                lo, hi = vs[g], vs[g | s]
                vs[g] = jnp.where(m, pltpu.roll(hi, s, 0), lo)
                vs[g | s] = jnp.where(m, hi, pltpu.roll(lo, 8 - s, 0))
    return vs


def build(DQK=0, DV=1, DO=1, RT=512, SLAB=48, HJ=1, AJ=16, WL=3, WH=2, NI=0, LD=2, EI=0, EO=0, GS=200, OT=1, PH=3, VW=5, PK=1, KD=3, S1=5, S2=2, S3=2, S4=4, OP=1, PV=1, N2=0, XP=1, EM=64, FLAG='', OJ=7):
    WEIGHTS = (WL, WH, WL, WL, WH, WH, WH)
    deep_t = (DQK, DQK, DV)
    nq = lambda deep: 7 if deep else 4
    XDEEP = 1 if all(deep_t) else 2
    PLAIN = (2, 7, 8, 3)

    def kern(zero_ref, x_hbm, wqkv_hbm, wo_hbm, wg_hbm, wu_hbm, wd_hbm, out_hbm,
             x_v, h_v, td, tq, tk, tv, to, sems, *bufs):
        xa = bufs[:7]
        td32, to32 = td.bitcast(u32), to.bitcast(u32)
        xa32 = [r.bitcast(u32) for r in xa]
        tqkv = (tq, tk, tv)
        def start(cps):
            for cp in cps:
                cp.start()

        def wait(cps):
            for cp in cps:
                cp.wait()

        zero = zero_ref[0]

        def opaque(ref):
            return ref.at[pl.ds(zero, ref.shape[0])]

        new_inner = dict
        new_states = lambda b=0: [{} for s in range(4)]

        def pacer(ref):
            r32 = ref.bitcast(f32)
            n = 8 if ref.dtype == f32 else 4
            idx = (0,) * (len(ref.shape) - 2) + (pl.ds(pl.multiple_of(r32.shape[-2] - 8 + zero, 8), n), pl.ds(0, L))

            def pace(v):
                r32[idx] = v[:n]
            return pace

        def operand_jobs(src, terms, deep, get, put):
            pace = pacer(src)

            def job(p):
                for q, v in enumerate(operands(terms, deep, p, get)):
                    put(p, q, v.astype(bf16))
            return [(pace, part(job, p)) for p in ORDER]

        def phase1(xn, raw_gu, raw_d, raw_d6, raw_qkv, mid_qkv, raw_o, mid_o, *tgu):
            tgu32 = [opaque(r.bitcast(u32)) if OT else r.bitcast(u32) for r in tgu]
            def x_copy(r):
                rows = pl.ds(pl.multiple_of(r * TM, TM), TM)
                return pltpu.make_async_copy(x_hbm.at[rows], x_v.at[rows], sems.at[r])

            def gu0_copies(o):
                rows, cols = pl.ds((o // 2) * 2 * QK, 2 * QK), pl.ds((o % 2) * 2 * L, 2 * L)
                return [pltpu.make_async_copy(w.at[rows, cols], raw_gu.at[0, t, rows, cols], sems.at[8 + o])
                        for t, w in enumerate((wg_hbm, wu_hbm))]

            def gu_copies(c):
                slot = c % 3
                cols = pl.ds(pl.multiple_of(c * 4 * L, 4 * L), 4 * L)
                return [pltpu.make_async_copy(w.at[:, cols], raw_gu.at[slot, t, pl.ds(0, D)], sems.at[12 + slot])
                        for t, w in enumerate((wg_hbm, wu_hbm))]

            def slab_row(it):
                return pl.multiple_of(jnp.minimum(it * SLAB, QK - SLAB), 16)

            def side_copies(it):
                slot = it & 1
                sem = sems.at[15 + slot]
                cps = [pltpu.make_async_copy(wd_hbm.at[pl.ds(pl.multiple_of(it * 4 * L, 4 * L), 4 * L)],
                                             raw_d.at[slot, pl.ds(0, 4 * L)], sem)]
                r0 = slab_row(it)
                for i in range(4):
                    cps.append(pltpu.make_async_copy(wqkv_hbm.at[pl.ds(i * QK + r0, SLAB)], raw_qkv.at[slot, i, pl.ds(0, SLAB)], sem))
                u = jnp.minimum(it, 3)
                rows = pl.ds(pl.multiple_of((u >> 1) * 512, 512), 512)
                for j in range(4):
                    cols = pl.ds(pl.multiple_of((2 * j + (u & 1)) * L, L), L)
                    cps.append(pltpu.make_async_copy(wo_hbm.at[rows, cols], raw_o.at[slot, j, pl.ds(0, 512)], sem))
                return cps

            d6_copy = pltpu.make_async_copy(wd_hbm.at[pl.ds((NCH - 1) * 4 * L, 4 * L)], raw_d6.at[pl.ds(0, 4 * L)], sems.at[17])

            x_copy(0).start()
            x_copy(1).start()
            for o in (0, 2, 3, 1):
                start(gu0_copies(o))
            for r in range(2, NT):
                x_copy(r).start()
            start(gu_copies(1) + gu_copies(2) + side_copies(0) + [d6_copy])
            def norm_jobs(r):
                mean, rstd = {}, {}
                load = lambda u, z: x_v[rows16(r * TM + u * 16 + z), :].astype(f32)

                def first(u):
                    mean[u] = jnp.mean(load(u, 0), axis=-1, keepdims=True)

                def second(u):
                    xc = load(u, zero) - mean[u]
                    rstd[u] = jax.lax.rsqrt(jnp.mean(xc * xc, axis=-1, keepdims=True) + 1e-5)

                def third(u):
                    xn[rows16(u * 16), :] = (load(u, 2 * zero) - mean[u]) * rstd[u]

                n = TM // 16
                return [(pacer(x_v), part(fn, u - k * LD)) for u in range(n + 2 * LD)
                        for k, fn in enumerate((first, second, third)) if 0 <= u - k * LD < n]

            def xa_jobs(r, ps=ORDER, p_major=True):
                def one(u, cg):
                    def put(p, q, v):
                        xa[p][r, q, cg, rows16(u * 16), :] = v
                    get = lambda i, j: xn[rows16(i * QR + u * 16 + zero), pl.ds((2 * j + cg) * L, L)]
                    return operand_jobs(xn, A_TERMS, XDEEP, get, put)
                jobs = [one(u, cg) for u in range(QR // 16) for cg in range(2)]
                if not p_major:
                    return [j[ORDER.index(p)] for j in jobs for p in ps]
                return [j[ORDER.index(p)] for p in ps for j in jobs]

            def gu_jobs(slot, p):
                def one(t, u):
                    def put(p, q, v):
                        tgu[p][q, t, rows16(u * 16), :] = v
                    get = lambda i, j: raw_gu[slot, t, rows16(i * QK + u * 16), pl.ds(j * L, L)].astype(f32)
                    return operand_jobs(raw_gu, B_TERMS, True, get, put)[ORDER.index(p)]
                return [one(t, u) for u in range(QK // 16) for t in range(2)]

            def wd_jobs(buf, src, r_src, r_dst, cg):
                def put(p, q, v):
                    td[p, q, cg, rows16(r_dst), :] = v
                get = lambda i, j: src[rows16(i * L + r_src), pl.ds((2 * j + cg) * L, L)].astype(f32)
                return operand_jobs(buf, B_TERMS, True, get, put)

            def qkv_permute(slot, t, u, i):
                cols = [pltpu.bitcast(raw_qkv[slot, i, rows16(u * 16), pl.ds(t * D + g * L, L)], u32) for g in range(8)]
                for g, c in enumerate(interleave_heads(cols)):
                    mid_qkv.bitcast(u32)[t * 8 + g, pl.ds((i * SLAB + u * 16) // 2, 8), :] = c

            def qkv_jobs(r0, t, u, cg):
                def put(p, q, v):
                    tqkv[t][p, q, cg, rows16(r0 + u * 16), :] = v
                get = lambda i, j: opaque(mid_qkv)[t * 8 + 2 * j + cg, rows16(i * SLAB + u * 16), :].astype(f32)
                return operand_jobs(mid_qkv, B_TERMS, deep_t[t], get, put)

            def wo_permute(slot, j, i, g1):
                old = [raw_o[slot, j, rows16(g1 * 256 + s * 32 + (i // 2) * 16), :].astype(f32)[(i % 2) * 8:(i % 2 + 1) * 8] for s in range(8)]
                for a, v in enumerate(transpose8(old)):
                    mid_o[j, pl.ds(i * L + a * 16 + g1 * 8, 8), :] = v

            def wo_jobs(unit, a):
                def put(p, q, v):
                    to[p, q, unit & 1, rows16(a * 32 + (unit >> 1) * 16), :] = v
                return operand_jobs(mid_o, B_TERMS, DO, lambda i, j: opaque(mid_o)[j ^ 2, rows16(i * L + a * 16), :], put)

            def gu_product(c, states, p, tiles, side):
                def sink(i, j, gu):
                    hh = geglu2(gu[:, :L], gu[:, L:]).astype(bf16)
                    for b, r in enumerate(tiles):
                        h_v[c, j, pl.ds(pl.multiple_of(r * TM + i * QR, QR), QR), :] = hh[b * QR:(b + 1) * QR]

                inner_product(True,
                              lambda q: cat([cat([xa32[p][r + zero, q, cg] for cg in range(2)], 1) for r in tiles], 0),
                              lambda q: cat([tgu32[p][q, t] for t in range(2)], 1),
                              outer_emit(states, p, sink), side, False, new_inner())


            def run(jobs):
                for _, job in jobs:
                    job()

            idle = [(None, lambda: None)]
            spaced = lambda jobs, n: [j for job in jobs for j in [job] + idle * n]

            states = [new_states(0), new_states(1)]

            def first(p, tiles, jobs):
                side = Side(jobs, 56 * len(tiles) - 24)
                for r in tiles:
                    gu_product(0, states[r], p, [r], side)

            mix = lambda a, b: [j for k in range(8) for j in a[k * len(a) // 8:(k + 1) * len(a) // 8] + b[k * len(b) // 8:(k + 1) * len(b) // 8]]
            g = lambda n: gu_jobs(0, ORDER[n])

            @pl.loop(0, 2)
            def _(r):
                x_copy(r).wait()
                if N2:
                    for u in range(TM // 16):
                        x = x_v[rows16(r * TM + u * 16), :].astype(f32)
                        xc = x - jnp.mean(x, axis=-1, keepdims=True)
                        xn[rows16(u * 16), :] = xc * jax.lax.rsqrt(jnp.mean(xc * xc, axis=-1, keepdims=True) + 1e-5)
                else:
                    run(norm_jobs(r))
                run(xa_jobs(r, p_major=False))
            wait(gu0_copies(0))
            nj = norm_jobs(2)
            if PV == 0:
                run(g(0))
                first(ORDER[0], [0], [])
                wait(gu0_copies(2))
                first(ORDER[0], [1], g(1))
                first(ORDER[1], [0], [])
                wait(gu0_copies(3))
                first(ORDER[1], [1], g(2))
                first(ORDER[2], [0, 1], g(3) + g(4)[:16])
            else:
                run(g(0))
                wait(gu0_copies(2))
                first(ORDER[0], [0, 1], g(1))
                wait(gu0_copies(3))
                first(ORDER[1], [0, 1], g(2))
                first(ORDER[2], [0, 1], g(3) + g(4)[:16])
            wait(gu0_copies(1))
            x_copy(2).wait()
            first(ORDER[3], [0, 1], mix(g(4)[16:] + g(5)[:16], nj[:16]))
            first(ORDER[4], [0, 1], mix(g(5)[16:] + g(6)[:8], nj[16:24]))
            first(ORDER[5], [0, 1], mix(g(6)[8:], nj[24:32]))
            first(ORDER[6], [0, 1], nj[32:] + xa_jobs(2, ORDER[:XP]))

            def chunk0_tile(r, _):
                @pl.when(r + 1 < NT)
                def _():
                    x_copy(r + 1).wait()

                nxt = jnp.minimum(r + 1, NT - 1)
                jobs = xa_jobs(r, ORDER[XP:]) + norm_jobs(nxt) + idle * NI + xa_jobs(nxt, ORDER[:XP])
                side = Side(jobs, 56 * sum(WEIGHTS) - 8 * WH)
                states = new_states()
                for n, p in enumerate(ORDER):
                    gu_product(0, states, p, [r], part(side, weight=WEIGHTS[n]))
                return 0

            jax.lax.fori_loop(2, NT, chunk0_tile, 0)
            wait(gu_copies(1))
            d6_copy.wait()
            run(gu_jobs(1, ORDER[0]))

            def chunk(c, _):
                it = c - 1
                slot = it & 1

                @pl.when(c + 1 < NCH)
                def _():
                    wait(gu_copies(c + 1))

                wait(side_copies(it))
                for cp in side_copies(it + 1):
                    pl.when(c + 1 < NCH)(cp.start)
                for cp in gu_copies(c + 2):
                    pl.when(c + 2 < NCH)(cp.start)
                r0 = slab_row(it)
                r6 = pl.multiple_of(jnp.minimum(it * 32, L - 32), 16)
                jobs = []
                for cg in range(2):
                    for u in range(L // 16):
                        jobs += wd_jobs(raw_d, raw_d.at[slot], u * 16, it * L + u * 16, cg)
                    for u in range(2):
                        jobs += wd_jobs(raw_d6, raw_d6, r6 + u * 16, (NCH - 1) * L + r6 + u * 16, cg)
                perm = [(pacer(raw_qkv), part(qkv_permute, slot, t, u, i)) for t in range(3) for u in range(SLAB // 16) for i in range(4)]
                for n, job in enumerate(perm):
                    jobs.insert(n * 4, job)
                jobs += [(pacer(raw_o), part(wo_permute, slot, j, i, g1)) for j in range(4) for i in range(4) for g1 in range(2)]
                for t in range(3):
                    for u in range(SLAB // 16):
                        for cg in range(2):
                            jobs += qkv_jobs(r0, t, u, cg)
                for a in range(8):
                    jobs += wo_jobs(jnp.minimum(it, 3), a)
                nb = RT // QR
                nrt = NT // nb
                per_p = 7 * S // 4 // 8
                weights = WEIGHTS
                extra = Side(jobs, sum(weights) * per_p - 32 * WH)
                states = [new_states(b) for b in range(nrt)]
                for n, p in enumerate(ORDER):
                    nxt = (c % 3, ORDER[n + 1]) if n < 6 else (jnp.minimum(c + 1, NCH - 1) % 3, ORDER[0])
                    side = Side(gu_jobs(*nxt), per_p - GS)

                    def both(v, side=side, wt=weights[n]):
                        side(v)
                        extra(v, wt)
                    for b in range(nrt):
                        gu_product(c, states[b], p, range(b * nb, (b + 1) * nb), both)
                return 0

            jax.lax.fori_loop(1, NCH, chunk, 0)

        def phase2(ha, q_sc, k_sc, v_sc, g_sc, obuf, *oa):
            def out_copy(r, o):
                rows, cols = (o // 2) * 2 * QR, pl.ds((o % 2) * 2 * QK, 2 * QK)
                return pltpu.make_async_copy(obuf.at[(r & 1), pl.ds(rows, 2 * QR), cols],
                                             out_hbm.at[pl.ds(pl.multiple_of(r * TM + rows, 2 * QR), 2 * QR), cols], sems.at[18 + (r & 1)])

            for g in range(8):
                k_sc[g, pl.ds(TM, HALO), :] = jnp.zeros((HALO, L), f32)
                v_sc[g, pl.ds(TM, HALO), :] = jnp.zeros((HALO, L), f32)

            def matmul(deep, lhs, rhs, sink, side, col_major):
                states = new_states()
                for n, p in enumerate(ORDER):
                    inner_product(deep, part(lhs, p), part(rhs, p), outer_emit(states, p, sink),
                                  side[n] if isinstance(side, list) else side, col_major, new_inner())

            def tile(r, _):
                @pl.when(r >= 2)
                def _():
                    wait([out_copy(r - 2, o) for o in range(4)])

                base = pl.multiple_of(r * TM, TM)
                for g in range(8):
                    k_sc[g, pl.ds(0, HALO), :] = k_sc[g, pl.ds(TM, HALO), :]
                    v_sc[g, pl.ds(0, HALO), :] = v_sc[g, pl.ds(TM, HALO), :]

                def h_jobs(c, u):
                    def put(p, q, v):
                        ha[p, q, c, rows16(u * 16), :] = v
                    jobs = operand_jobs(h_v, A_TERMS, True, lambda i, j: h_v[c, j, rows16(base + i * QR + u * 16), :].astype(f32), put)
                    if HJ:
                        return jobs
                    return [(jobs[0][0], lambda: [job() for _, job in jobs])]

                att = {}
                q_d, k_d, v_d, g_d = (opaque(ref) for ref in (q_sc, k_sc, v_sc, g_sc))

                def logits(r0, w):
                    k_sc[8 + w, pl.ds(r0, AJ), :] = functools.reduce(
                        jnp.add, [q_d[g, pl.ds(r0, AJ), :] * k_d[g, pl.ds(r0 + HALO - DIL * w, AJ), :] for g in range(8)])

                def rotate(r0, w):
                    l = k_d[8 + w, pl.ds(r0, AJ), :]
                    att[r0, w] = [pltpu.roll(l, s, 1) for s in (32, 64, 96)]

                def fold(r0, w):
                    l = functools.reduce(jnp.add, att[r0, w], k_d[8 + w, pl.ds(r0, AJ), :])
                    if r0 < HALO and w > 0:
                        pos = base + r0 + jax.lax.broadcasted_iota(jnp.int32, (AJ, L), 0)
                        l = jnp.where(pos >= DIL * w, l, -1e9 * LOG2E)
                    att[r0, w] = l

                def unfold(r0, w):
                    k_sc[8 + w, pl.ds(r0, AJ), :] = att[r0, w]

                def softmax(r0):
                    ls = [k_d[8 + w, pl.ds(r0, 8), :] for w in range(W)]
                    mx = functools.reduce(jnp.maximum, ls)
                    ps = [jnp.exp2(l - mx) for l in ls]
                    inv = 1.0 / functools.reduce(jnp.add, ps)
                    for w in range(W):
                        k_sc[8 + w, pl.ds(r0, 8), :] = ps[w] * inv

                def mix(r0, g):
                    v_sc[8 + g, pl.ds(r0, AJ), :] = functools.reduce(
                        jnp.add, [k_d[8 + w, pl.ds(r0, AJ), :] * v_d[g, pl.ds(r0 + HALO - DIL * w, AJ), :] for w in range(W)])

                def o_jobs(u, cg):
                    def put(p, q, v):
                        oa[p][q, cg, rows16(u * 16), :] = v
                    return operand_jobs(v_sc, A_TERMS, DO, lambda i, j: v_d[8 + 2 * j + cg, rows16(i * QR + u * 16), :], put)

                starts = list(range(0, TM, AJ))
                jobs = []
                idle = (None, lambda: None)
                cells = [(r0, w) for r0 in starts for w in range(W)]

                def step(n):
                    for fn, d in ((rotate, PK), (fold, PK + KD), (logits, 0), (unfold, PK + KD)):
                        if 0 <= n - d < len(cells):
                            fn(*cells[n - d])

                for n in range(len(cells) + PK + KD):
                    jobs += [(pacer(k_sc), part(step, n))] + [idle] * (S1 - 1)
                for r0 in range(0, TM, 8):
                    jobs += [(pacer(k_sc), part(softmax, r0))] + [idle] * (S4 - 1)
                jobs += [j for r0 in starts for g in range(8) for j in [(pacer(v_sc), part(mix, r0, g))] + [idle] * (S2 - 1)]
                oj = [o_jobs(u, cg) for u in range(QR // 16) for cg in range(2)]
                jobs += [k for n in range(OJ) for j in oj for k in [j[n]] + [idle] * (S3 - 1)]
                ticks = lambda deep: 49 * 8 if deep else 14 * 32
                wts = (5, 4, 5, 5, 4, 4, 4)
                attn = Side(jobs, VW * ticks(DV) + 7 * 16 * sum(wts) - EM * 4)
                side = Side([j for c in range(NCH) for u in range(QR // 16) for j in h_jobs(c, u)],
                            2 * ticks(DQK) * 8 + (8 - VW) * ticks(DV) - 160)
                for t, dst, off in ((1, k_sc, HALO), (0, q_sc, 0), (2, v_sc, HALO)):
                    def sink(i, j, val, t=t, dst=dst, off=off):
                        if t == 0:
                            val = val * (DH ** -0.5 * LOG2E)
                        for cg in range(2):
                            dst[2 * j + cg, pl.ds(off + i * QR, QR), :] = val[:, cg * L:(cg + 1) * L]
                            if t == 2 and i == 0:
                                halo = dst[2 * j + cg, pl.ds(0, HALO), :]
                                first = jnp.broadcast_to(val[0:1, cg * L:(cg + 1) * L], (HALO, L))
                                dst[2 * j + cg, pl.ds(0, HALO), :] = jnp.where(r == 0, first, halo)
                    t32 = tqkv[t].bitcast(u32)
                    deep = deep_t[t]
                    matmul(deep,
                           lambda p, q: cat([xa32[p][r, q if deep else PLAIN[q], cg] for cg in range(2)], 1),
                           lambda p, q: cat([t32[p, q, cg] for cg in range(2)], 1), sink,
                           part(side, weight=8) if t < 2 else lambda v: (side(v, 8 - VW), attn(v, VW)), not deep)
                side = [part(attn, weight=w) for w in wts]

                def y_sink(i, j, val):
                    y2 = val * 0.25
                    gt = y2 * jnp.tanh(y2) + y2
                    for cg in range(2):
                        g_sc[2 * j + cg, pl.ds(i * QR, QR), :] = gt[:, cg * L:(cg + 1) * L]

                ha32, oa32 = opaque(ha.bitcast(u32)), [opaque(a.bitcast(u32)) for a in oa]
                matmul(True,
                       lambda p, q: cat([ha32[p, q, c] for c in range(NCH)], 1),
                       lambda p, q: cat([td32[p, q, cg] for cg in range(2)], 1), y_sink, side, True)

                pending = [4] * 4

                def s_sink(i, j, val):
                    j ^= 2
                    cols = pl.ds(j * QK, QK)
                    xs = x_v[pl.ds(base + i * QR, QR), cols].astype(f32)
                    gate = cat([g_d[2 * j + cg, pl.ds(i * QR, QR), :] for cg in range(2)], 1)
                    obuf[(r & 1), pl.ds(i * QR, QR), cols] = (xs + val * gate).astype(bf16)
                    o = 2 * (i // 2) + j // 2
                    pending[o] -= 1
                    if not pending[o]:
                        out_copy(r, o).start()

                matmul(DO,
                       lambda p, q: cat([oa32[p][q, cg] for cg in range(2)], 1),
                       lambda p, q: cat([to32[p, q, cg] for cg in range(2)], 1), s_sink,
                       [Side([j[n + OJ] for j in oj] if n + OJ < 7 else [], 48 if OJ > 1 else 24, OP) for n in range(7)], False)
                return 0

            jax.lax.fori_loop(0, NT, tile, 0)
            wait([out_copy(r, o) for r in (NT - 2, NT - 1) for o in range(4)])

        if PH & 1:
            phase1(*bufs[7:22])
        if PH == 1:
            for b in (td, tq, tk, tv, to):
                pltpu.sync_copy(b.at[zero, 0, 0, pl.ds(0, 16)], out_hbm.at[pl.ds(0, 16), pl.ds(0, L)])
            pltpu.sync_copy(h_v.at[zero, 0, pl.ds(0, 16)], out_hbm.at[pl.ds(0, 16), pl.ds(0, L)])
        if PH & 2:
            phase2(*bufs[22:])

    def fn(A_x, A_wqkv, A_wo, B_x, B_w_gate, B_w_up, B_w_down):
        any_spec = pl.BlockSpec(memory_space=pl.ANY)
        V = pltpu.VMEM
        dma = pltpu.SemaphoreType.DMA
        out = pl.pallas_call(
            kern,
            in_specs=[pl.BlockSpec(memory_space=pltpu.SMEM)] + [any_spec] * 6,
            out_specs=any_spec,
            out_shape=jax.ShapeDtypeStruct((S, D), A_x.dtype),
            scratch_shapes=[
                V((S + PAD, D), bf16), V((NCH, 4, S + PAD, L), bf16),
                V((7, 7, 2, F // 4, L), bf16),
                V((7, nq(DQK), 2, QK, L), bf16), V((7, nq(DQK), 2, QK, L), bf16), V((7, nq(DV), 2, QK, L), bf16),
                V((7, nq(DO), 2, QK, L), bf16),
                dma((20,)), *[V((NT, 5 + 2 * XDEEP, 2, QR, L), bf16)] * 7,
                V((TM + PAD, D), f32),
                V((3, 2, D + PAD, 4 * L), bf16), V((2, 4 * L + PAD, D), bf16), V((4 * L + PAD, D), bf16),
                V((2, 4, SLAB + PAD, 3 * D), bf16), V((24, 4 * SLAB + PAD, L), bf16),
                V((2, 4, 512 + PAD, L), bf16), V((4, 512 + PAD, L), f32), *[V((7, 2, QK, L), bf16)] * 7,
                V((7, 7, NCH, QR, L), bf16),
                V((8, TM, L), f32), V((16, TM + HALO + PAD, L), f32), V((16, TM + HALO + PAD, L), f32),
                V((8, TM, L), f32), V((2, TM, D), bf16), *[V((nq(DO), 2, QR, L), bf16)] * 7,
            ],
            compiler_params=pltpu.CompilerParams(vmem_limit_bytes=127 * 1024 * 1024, disable_bounds_checks=True, flags={FLAG: True} if FLAG else None),
        )(jnp.zeros((1,), jnp.int32), A_x.reshape(S, D), A_wqkv, A_wo, B_w_gate, B_w_up, B_w_down)
        return out.reshape(A_x.shape)

    return fn


pallas_recurrent_scan__sliding_local_dilated__geglu_ffn__prompt_kernel = jax.jit(build())
```

```python
import functools

import jax
import jax.numpy as jnp
import jax.experimental.pallas as pl
import jax.experimental.pallas.tpu as pltpu

S, D, F = 2048, 1024, 3584
DH, W, DIL = 32, 8, 2
L = 128
TM = 256
QR = TM // 4
NT = S // TM
QK = D // 4
CW = 4 * L
NCH = F // CW
HALO = 16
SLAB = 48
PAD = 16
LOG2E = 1.4426950408889634
f32, bf16, u32 = jnp.float32, jnp.bfloat16, jnp.uint32
part = functools.partial

A_TERMS = ((0, 1, 3), (2, 1, 3), (0,), (3,), (0, 1, 1), (2, -1, 0), (1, -1, 3))
B_TERMS = ((0, 1, 3), (0,), (1, -1, 3), (2, -1, 0), (3,), (0, 1, 1), (2, 1, 3))
C_TERMS = (((0, 1), (3, 1)), ((2, 1), (3, -1)), ((1, 1), (3, 1)), ((0, 1), (2, 1)),
           ((0, -1), (1, 1)), ((3, 1),), ((0, 1),))
C_COUNT = (4, 2, 2, 4)
OUTER = (1, 3, 4, 0, 6, 2, 5)
INNER = (1, 3, 0, 6, 4, 2, 5)
LOAD = (3, 2, 3, 3, 2, 2, 2)
FLIP = (0, 1, 0, 0, 1, 1, 1)
PLAIN, DEEP, BOTH = 4, 7, 9
PLAIN_IN_BOTH = (2, 7, 8, 3)
QKV_SPLIT = (PLAIN, PLAIN, DEEP)


def _lin(term, get):
    if len(term) == 1:
        return get(term[0])
    a, b = get(term[0]), get(term[2])
    return a + b if term[1] > 0 else a - b


def _operands(terms, split, p, get):
    flip = FLIP[p] if terms is B_TERMS else 0
    blk = [_lin(terms[p], lambda o: get(2 * (o // 2) + s // 2, 2 * (o % 2) + (s % 2 ^ flip))) for s in range(4)]
    if split == PLAIN:
        return blk
    return [_lin(t, lambda s: blk[s]) for t in terms] + ([blk[1], blk[2]] if split == BOTH else [])


def _combine(state, p, m):
    done = []
    for o, sign in C_TERMS[p]:
        if o in state:
            n, s0, acc = state[o]
            assert s0 > 0 or sign > 0
            acc = acc + m if s0 == sign else (acc - m if s0 > 0 else m - acc)
            state[o] = (n + 1, 1, acc)
            if n + 1 == C_COUNT[o]:
                done.append((o, acc))
        else:
            state[o] = (1, sign, m)
    return done


def _cat(xs, axis):
    return xs[0] if len(xs) == 1 else jnp.concatenate(xs, axis)


def _mxu(a, b):
    return jnp.dot(pltpu.bitcast(a, bf16), pltpu.bitcast(b, bf16), preferred_element_type=f32)


def _outer_product(split, p, states, lhs, rhs, sink, tick, tick_cols):
    def emit(s, m):
        s ^= FLIP[p]
        for o, val in _combine(states[s], p, m):
            sink(2 * (o // 2) + s // 2, 2 * (o % 2) + s % 2, val)

    def ticks(m):
        for b in range(tick_cols):
            for r in range(m.shape[0] // 8):
                tick(m, r, b)

    if split == DEEP:
        inner = {}
        for q in INNER:
            m = _mxu(lhs(q), rhs(q))
            for s, val in _combine(inner, q, m):
                emit(s, val)
            ticks(m)
    else:
        a = _cat([_cat([lhs(0), lhs(1)], 1), _cat([lhs(2), lhs(3)], 1)], 0)
        for j in range(2):
            m = _mxu(a, _cat([rhs(j), rhs(2 + j)], 0))
            n = m.shape[0] // 2
            emit(j, m[:n])
            emit(2 + j, m[n:])
            ticks(m)


class _Side:
    def __init__(self, jobs, span):
        self.jobs, self.span, self.n, self.done = list(jobs), span, 0, 0

    def __call__(self, m, r, b, weight=1):
        self.n += weight
        while self.done < len(self.jobs) and self.done * self.span < self.n * len(self.jobs):
            if self.jobs[self.done] is not None:
                pace, job = self.jobs[self.done]
                pace(m[r * 8:(r + 1) * 8, b * L:(b + 1) * L])
                job()
            self.done += 1

    def check(self):
        assert self.done == len(self.jobs)


def _spaced(jobs, n):
    return [j for job in jobs for j in [job] + [None] * (n - 1)]


def _merged(a, b):
    cut = lambda v, k: v[k * len(v) // 8:(k + 1) * len(v) // 8]
    return [j for k in range(8) for j in cut(a, k) + cut(b, k)]


def _run(jobs):
    for _, job in jobs:
        job()


def _rows(r, n=16):
    return pl.ds(r if isinstance(r, int) else pl.multiple_of(r, n), n)


def _words(ref):
    return ref.bitcast(u32)


def _geglu2(g, u):
    c = 0.7978845608028654
    th = jnp.tanh(g * (g * g * (c * 0.044715) + c))
    a = g * u
    return a * th + a


def _interleave_heads(cols):
    cols = list(cols)
    lane = jax.lax.broadcasted_iota(jnp.int32, cols[0].shape, 1)
    for b in range(3):
        s = 4 << b
        m = (lane & s) != 0
        for g in range(8):
            if not g & (1 << b):
                lo, hi = cols[g], cols[g | (1 << b)]
                cols[g] = jnp.where(m, pltpu.roll(hi, s, 1), lo)
                cols[g | (1 << b)] = jnp.where(m, hi, pltpu.roll(lo, L - s, 1))
    idx = (lane & 0x1C) | ((lane & 3) << 5) | (lane >> 5)
    return [jnp.take_along_axis(c, idx, axis=1) for c in cols]


def _transpose8(vs):
    vs = list(vs)
    sub = jax.lax.broadcasted_iota(jnp.int32, vs[0].shape, 0)
    for s in (1, 2, 4):
        m = (sub & s) != 0
        for g in range(8):
            if not g & s:
                lo, hi = vs[g], vs[g | s]
                vs[g] = jnp.where(m, pltpu.roll(hi, s, 0), lo)
                vs[g | s] = jnp.where(m, hi, pltpu.roll(lo, 8 - s, 0))
    return vs


def _start(copies):
    for cp in copies:
        cp.start()


def _wait(copies):
    for cp in copies:
        cp.wait()


def _kernel(zero_ref, x_hbm, wqkv_hbm, wo_hbm, wg_hbm, wu_hbm, wd_hbm, out_hbm,
            x_v, h_v, td, tq, tk, tv, to, sems, xa,
            xn, raw_gu, raw_d, raw_d6, raw_qkv, mid_qkv, raw_o, mid_o, tgu,
            ha, q_v, k_v, v_v, g_v, obuf, oa):
    zero = zero_ref[0]
    tqkv = (tq, tk, tv)
    new_states = lambda: [{} for _ in range(4)]

    def opaque(ref):
        return ref.at[pl.ds(zero, ref.shape[0])]

    def pacer(ref):
        def pace(v):
            v = pltpu.bitcast(v, u32) if ref.dtype == u32 else v.astype(ref.dtype)
            ref[(0,) * (len(ref.shape) - 2) + (_rows(ref.shape[-2] - 8 + zero, 8), pl.ds(0, L))] = v
        return pace

    def operand_jobs(src, terms, split, get, put):
        def job(p):
            for q, v in enumerate(_operands(terms, split, p, get)):
                put(p, q, v.astype(bf16))
        return [(pacer(src), part(job, p)) for p in OUTER]

    def x_copy(r):
        return pltpu.make_async_copy(x_hbm.at[_rows(r * TM, TM)], x_v.at[_rows(r * TM, TM)], sems.at[r])

    def gu0_copies(o):
        rows, cols = pl.ds((o // 2) * 2 * QK, 2 * QK), pl.ds((o % 2) * 2 * L, 2 * L)
        return [pltpu.make_async_copy(w.at[rows, cols], raw_gu.at[0, t, rows, cols], sems.at[8 + o])
                for t, w in enumerate((wg_hbm, wu_hbm))]

    def gu_copies(c):
        return [pltpu.make_async_copy(w.at[:, _rows(c * CW, CW)], raw_gu.at[c % 3, t, pl.ds(0, D)], sems.at[12 + c % 3])
                for t, w in enumerate((wg_hbm, wu_hbm))]

    def side_copies(it):
        slot, unit = it & 1, jnp.minimum(it, 3)
        sem = sems.at[15 + slot]
        r0 = pl.multiple_of(jnp.minimum(it * SLAB, QK - SLAB), 16)
        return ([pltpu.make_async_copy(wd_hbm.at[_rows(it * CW, CW)], raw_d.at[slot, pl.ds(0, CW)], sem)]
                + [pltpu.make_async_copy(wqkv_hbm.at[pl.ds(i * QK + r0, SLAB)], raw_qkv.at[slot, i, pl.ds(0, SLAB)], sem)
                   for i in range(4)]
                + [pltpu.make_async_copy(wo_hbm.at[_rows((unit >> 1) * 2 * QK, 2 * QK), _rows((2 * j + (unit & 1)) * L, L)],
                                         raw_o.at[slot, j, pl.ds(0, 2 * QK)], sem) for j in range(4)])

    def d6_copy():
        return pltpu.make_async_copy(wd_hbm.at[pl.ds((NCH - 1) * CW, CW)], raw_d6.at[pl.ds(0, CW)], sems.at[17])

    _start([x_copy(0), x_copy(1)] + [cp for o in (0, 2, 3, 1) for cp in gu0_copies(o)]
           + [x_copy(r) for r in range(2, NT)] + gu_copies(1) + gu_copies(2) + side_copies(0) + [d6_copy()])

    def norm_jobs(r):
        mean, rstd = {}, {}
        load = lambda u, z: x_v[_rows(r * TM + u * 16 + z), :].astype(f32)

        def centre(u):
            mean[u] = jnp.mean(load(u, 0), axis=-1, keepdims=True)

        def spread(u):
            xc = load(u, zero) - mean[u]
            rstd[u] = jax.lax.rsqrt(jnp.mean(xc * xc, axis=-1, keepdims=True) + 1e-5)

        def scale(u):
            xn[_rows(u * 16), :] = (load(u, 2 * zero) - mean[u]) * rstd[u]

        n = TM // 16
        return [(pacer(x_v), part(fn, u - 2 * k)) for u in range(n + 4)
                for k, fn in enumerate((centre, spread, scale)) if 0 <= u - 2 * k < n]

    def xa_jobs(r):
        def one(u, cg):
            def put(p, q, v):
                xa[p][r, q, cg, _rows(u * 16), :] = v
            get = lambda i, j: xn[_rows(i * QR + u * 16 + zero), pl.ds((2 * j + cg) * L, L)]
            return operand_jobs(xn, A_TERMS, BOTH, get, put)
        return [one(u, cg) for u in range(QR // 16) for cg in range(2)]

    def gu_jobs(slot, n):
        def one(u, t):
            def put(p, q, v):
                tgu[p][q, t, _rows(u * 16), :] = v
            get = lambda i, j: raw_gu[slot, t, _rows(i * QK + u * 16), pl.ds(j * L, L)].astype(f32)
            return operand_jobs(raw_gu, B_TERMS, DEEP, get, put)[n]
        return [one(u, t) for u in range(QK // 16) for t in range(2)]

    def wd_jobs(buf, lead, r_src, r_dst, cg):
        def put(p, q, v):
            td[p, q, cg, _rows(r_dst), :] = v
        get = lambda i, j: buf[lead + (_rows(i * L + r_src), pl.ds((2 * j + cg) * L, L))].astype(f32)
        return operand_jobs(buf, B_TERMS, DEEP, get, put)

    def qkv_permute(slot, t, u, i):
        cols = [pltpu.bitcast(raw_qkv[slot, i, _rows(u * 16), pl.ds(t * D + g * L, L)], u32) for g in range(8)]
        for g, c in enumerate(_interleave_heads(cols)):
            mid_qkv[t * 8 + g, _rows((i * SLAB + u * 16) // 2, 8), :] = c

    def qkv_jobs(r0, t, u, cg):
        def put(p, q, v):
            tqkv[t][p, q, cg, _rows(r0 + u * 16), :] = v
        get = lambda i, j: pltpu.bitcast(
            opaque(mid_qkv)[t * 8 + 2 * j + cg, _rows((i * SLAB + u * 16) // 2, 8), :], bf16).astype(f32)
        return operand_jobs(mid_qkv, B_TERMS, QKV_SPLIT[t], get, put)

    def wo_permute(slot, j, i, g1):
        old = [raw_o[slot, j, _rows(g1 * QK + s * DH + (i // 2) * 16), :].astype(f32)[(i % 2) * 8:(i % 2 + 1) * 8]
               for s in range(8)]
        for a, v in enumerate(_transpose8(old)):
            mid_o[j, _rows(i * L + a * 16 + g1 * 8, 8), :] = v

    def wo_jobs(unit, a):
        def put(p, q, v):
            to[p, q, unit & 1, _rows(a * 32 + (unit >> 1) * 16), :] = v
        return operand_jobs(mid_o, B_TERMS, DEEP, lambda i, j: opaque(mid_o)[j ^ 2, _rows(i * L + a * 16), :], put)

    def gu_product(c, states, n, tiles, tick):
        p = OUTER[n]

        def sink(i, j, gu):
            h = _geglu2(gu[:, :L], gu[:, L:]).astype(bf16)
            for b, r in enumerate(tiles):
                h_v[c, j, _rows(r * TM + i * QR, QR), :] = h[b * QR:(b + 1) * QR]

        _outer_product(DEEP, p, states,
                       lambda q: _cat([_cat([_words(xa[p])[r + zero, q, cg] for cg in range(2)], 1) for r in tiles], 0),
                       lambda q: _cat([opaque(_words(tgu[p]))[q, t] for t in range(2)], 1), sink, tick, 1)

    @pl.loop(0, 2)
    def _(r):
        x_copy(r).wait()
        _run(norm_jobs(r) + [job for piece in xa_jobs(r) for job in piece])

    first_states = [new_states(), new_states()]

    def first(n, tiles, jobs):
        side = _Side(jobs, 56 * len(tiles) - 24)
        for r in tiles:
            gu_product(0, first_states[r], n, [r], side)
        side.check()

    g0 = part(gu_jobs, 0)
    _wait(gu0_copies(0))
    _run(g0(0))
    first(0, [0], [])
    _wait(gu0_copies(2))
    first(0, [1], g0(1))
    first(1, [0], [])
    _wait(gu0_copies(3))
    first(1, [1], g0(2))
    first(2, [0, 1], g0(3) + g0(4)[:16])
    _wait(gu0_copies(1) + [x_copy(2)])
    norm2 = norm_jobs(2)
    first(3, [0, 1], _merged(g0(4)[16:] + g0(5)[:16], norm2[:16]))
    first(4, [0, 1], _merged(g0(5)[16:] + g0(6)[:8], norm2[16:24]))
    first(5, [0, 1], _merged(g0(6)[8:], norm2[24:32]))
    first(6, [0, 1], norm2[32:] + [piece[0] for piece in xa_jobs(2)])

    @pl.loop(2, NT)
    def _(r):
        nxt = jnp.minimum(r + 1, NT - 1)
        pl.when(r + 1 < NT)(x_copy(nxt).wait)
        jobs = ([piece[n] for n in range(1, 7) for piece in xa_jobs(r)]
                + norm_jobs(nxt) + [piece[0] for piece in xa_jobs(nxt)])
        side = _Side(jobs, 56 * sum(LOAD) - 16)
        states = new_states()
        for n in range(7):
            gu_product(0, states, n, [r], part(side, weight=LOAD[n]))
        side.check()

    _wait(gu_copies(1) + [d6_copy()])
    _run(gu_jobs(1, 0))

    @pl.loop(1, NCH)
    def _(c):
        it = c - 1
        slot, nxt = it & 1, jnp.minimum(c + 1, NCH - 1)
        pl.when(c + 1 < NCH)(lambda: _wait(gu_copies(nxt)))
        _wait(side_copies(it))
        for cp in side_copies(c):
            pl.when(c + 1 < NCH)(cp.start)
        for cp in gu_copies(jnp.minimum(c + 2, NCH - 1)):
            pl.when(c + 2 < NCH)(cp.start)

        r0 = jnp.minimum(it * SLAB, QK - SLAB)
        r6 = jnp.minimum(it * 32, L - 32)
        jobs = []
        for cg in range(2):
            for u in range(L // 16):
                jobs += wd_jobs(raw_d, (slot,), u * 16, it * L + u * 16, cg)
            for u in range(2):
                jobs += wd_jobs(raw_d6, (), r6 + u * 16, (NCH - 1) * L + r6 + u * 16, cg)
        slabs = [(t, u) for t in range(3) for u in range(SLAB // 16)]
        for n, (t, u, i) in enumerate((t, u, i) for t, u in slabs for i in range(4)):
            jobs.insert(4 * n, (pacer(raw_qkv), part(qkv_permute, slot, t, u, i)))
        jobs += [(pacer(raw_o), part(wo_permute, slot, j, i, g1)) for j in range(4) for i in range(4) for g1 in range(2)]
        jobs += [job for t, u in slabs for cg in range(2) for job in qkv_jobs(r0, t, u, cg)]
        jobs += [job for a in range(8) for job in wo_jobs(jnp.minimum(it, 3), a)]
        per_product = 7 * NT * QR // 8
        extra = _Side(jobs, sum(LOAD) * per_product - 64)
        states = new_states()
        for n in range(7):
            side = _Side(gu_jobs(c % 3, n + 1) if n < 6 else gu_jobs(nxt % 3, 0), per_product - 200)
            gu_product(c, states, n, range(NT), lambda *a: (side(*a), extra(*a, weight=LOAD[n])))
            side.check()
        extra.check()

    def out_copies(r):
        def one(o):
            rows, cols = (o // 2) * 2 * QR, pl.ds((o % 2) * 2 * QK, 2 * QK)
            return pltpu.make_async_copy(obuf.at[r & 1, pl.ds(rows, 2 * QR), cols],
                                         out_hbm.at[_rows(r * TM + rows, 2 * QR), cols], sems.at[18 + (r & 1)])
        return [one(o) for o in range(4)]

    def project(split, lhs, rhs, sink, tick, tick_cols):
        states = new_states()
        for n, p in enumerate(OUTER):
            _outer_product(split, p, states, part(lhs, p), part(rhs, p), sink, part(tick, n), tick_cols)

    for g in range(8):
        k_v[g, pl.ds(TM, HALO), :] = jnp.zeros((HALO, L), f32)
        v_v[g, pl.ds(TM, HALO), :] = jnp.zeros((HALO, L), f32)

    @pl.loop(0, NT)
    def _(r):
        pl.when(r >= 2)(lambda: _wait(out_copies(r - 2)))
        for g in range(8):
            k_v[g, pl.ds(0, HALO), :] = k_v[g, pl.ds(TM, HALO), :]
            v_v[g, pl.ds(0, HALO), :] = v_v[g, pl.ds(TM, HALO), :]

        def h_jobs(c, u):
            def put(p, q, v):
                ha[p, q, c, _rows(u * 16), :] = v
            get = lambda i, j: h_v[c, j, _rows(r * TM + i * QR + u * 16), :].astype(f32)
            return operand_jobs(h_v, A_TERMS, DEEP, get, put)

        q_o, k_o, v_o, g_o = (opaque(ref) for ref in (q_v, k_v, v_v, g_v))
        window = lambda r0, w: pl.ds(r0 + HALO - DIL * w, 16)
        cells = [(r0, w) for r0 in range(0, TM, 16) for w in range(W)]
        held = {}

        def logits(r0, w):
            k_v[8 + w, _rows(r0), :] = functools.reduce(
                jnp.add, [q_o[g, _rows(r0), :] * k_o[g, window(r0, w), :] for g in range(8)])

        def rotate(r0, w):
            held[r0, w] = [pltpu.roll(k_o[8 + w, _rows(r0), :], s, 1) for s in (32, 64, 96)]

        def fold(r0, w):
            l = functools.reduce(jnp.add, held[r0, w], k_o[8 + w, _rows(r0), :])
            if r0 < HALO and w > 0:
                pos = r * TM + r0 + jax.lax.broadcasted_iota(jnp.int32, l.shape, 0)
                l = jnp.where(pos >= DIL * w, l, -1e9 * LOG2E)
            held[r0, w] = l

        def keep(r0, w):
            k_v[8 + w, _rows(r0), :] = held[r0, w]

        def logit_step(n):
            for fn, lag in ((rotate, 2), (fold, 6), (logits, 0), (keep, 6)):
                if 0 <= n - lag < len(cells):
                    fn(*cells[n - lag])

        def softmax(r0):
            ls = [k_o[8 + w, _rows(r0, 8), :] for w in range(W)]
            top = functools.reduce(jnp.maximum, ls)
            ps = [jnp.exp2(l - top) for l in ls]
            inv = 1.0 / functools.reduce(jnp.add, ps)
            for w in range(W):
                k_v[8 + w, _rows(r0, 8), :] = ps[w] * inv

        def mix(r0, g):
            v_v[8 + g, _rows(r0), :] = functools.reduce(
                jnp.add, [k_o[8 + w, _rows(r0), :] * v_o[g, window(r0, w), :] for w in range(W)])

        def o_jobs(u, cg):
            def put(p, q, v):
                oa[p][q, cg, _rows(u * 16), :] = v
            return operand_jobs(v_v, A_TERMS, DEEP, lambda i, j: v_o[8 + 2 * j + cg, _rows(i * QR + u * 16), :], put)

        pieces = [o_jobs(u, cg) for u in range(QR // 16) for cg in range(2)]
        attn = _Side(_spaced([(pacer(k_v), part(logit_step, n)) for n in range(len(cells) + 6)], 5)
                     + _spaced([(pacer(k_v), part(softmax, r0)) for r0 in range(0, TM, 8)], 4)
                     + _spaced([(pacer(v_v), part(mix, r0, g)) for r0 in range(0, TM, 16) for g in range(8)], 2)
                     + _spaced([piece[n] for n in range(7) for piece in pieces], 2),
                     5 * 392 + 112 * (sum(LOAD) + 14) - 256)
        side = _Side([job for c in range(NCH) for u in range(QR // 16) for job in h_jobs(c, u)],
                     8 * 896 + 3 * 392 - 160)

        for t, dst, off in ((1, k_v, HALO), (0, q_v, 0), (2, v_v, HALO)):
            def sink(i, j, val):
                if t == 0:
                    val = val * (DH ** -0.5 * LOG2E)
                for cg in range(2):
                    piece = val[:, cg * L:(cg + 1) * L]
                    dst[2 * j + cg, pl.ds(off + i * QR, QR), :] = piece
                    if t == 2 and i == 0:
                        dst[2 * j + cg, pl.ds(0, HALO), :] = jnp.where(
                            r == 0, jnp.broadcast_to(piece[0:1], (HALO, L)), dst[2 * j + cg, pl.ds(0, HALO), :])

            deep = QKV_SPLIT[t] == DEEP
            project(QKV_SPLIT[t],
                    lambda p, q: _cat([_words(xa[p])[r, q if deep else PLAIN_IN_BOTH[q], cg] for cg in range(2)], 1),
                    lambda p, q: _cat([_words(tqkv[t])[p, q, cg] for cg in range(2)], 1), sink,
                    (lambda n, *a: side(*a, weight=8)) if t < 2 else (lambda n, *a: (side(*a, weight=3), attn(*a, weight=5))),
                    1 if deep else 2)
        side.check()

        def gate_sink(i, j, val):
            half = val * 0.25
            gate = half * jnp.tanh(half) + half
            for cg in range(2):
                g_v[2 * j + cg, pl.ds(i * QR, QR), :] = gate[:, cg * L:(cg + 1) * L]

        project(DEEP, lambda p, q: _cat([opaque(_words(ha))[p, q, c] for c in range(NCH)], 1),
                lambda p, q: _cat([_words(td)[p, q, cg] for cg in range(2)], 1), gate_sink,
                lambda n, *a: attn(*a, weight=LOAD[n] + 2), 2)
        attn.check()

        copies, pending = out_copies(r), [4] * 4

        def out_sink(i, j, val):
            j ^= 2
            cols = pl.ds(j * QK, QK)
            gate = _cat([g_o[2 * j + cg, pl.ds(i * QR, QR), :] for cg in range(2)], 1)
            res = x_v[_rows(r * TM + i * QR, QR), cols].astype(f32) + val * gate
            obuf[r & 1, pl.ds(i * QR, QR), cols] = res.astype(obuf.dtype)
            o = 2 * (i // 2) + j // 2
            pending[o] -= 1
            if not pending[o]:
                copies[o].start()

        project(DEEP, lambda p, q: _cat([opaque(_words(oa[p]))[q, cg] for cg in range(2)], 1),
                lambda p, q: _cat([_words(to)[p, q, cg] for cg in range(2)], 1), out_sink, lambda *a: None, 0)

    _wait(out_copies(NT - 2) + out_copies(NT - 1))


@jax.jit
def pallas_recurrent_scan__sliding_local_dilated__geglu_ffn__prompt_kernel(
    A_x: jax.Array,
    A_wqkv: jax.Array,
    A_wo: jax.Array,
    B_x: jax.Array,
    B_w_gate: jax.Array,
    B_w_up: jax.Array,
    B_w_down: jax.Array,
):
    del B_x
    hbm = pl.BlockSpec(memory_space=pl.ANY)
    V = pltpu.VMEM
    out = pl.pallas_call(
        _kernel,
        in_specs=[pl.BlockSpec(memory_space=pltpu.SMEM)] + [hbm] * 6,
        out_specs=hbm,
        out_shape=jax.ShapeDtypeStruct((S, D), bf16),
        scratch_shapes=[
            V((S + PAD, D), bf16),
            V((NCH, 4, S + PAD, L), bf16),
            V((7, DEEP, 2, F // 4, L), bf16),
            *[V((7, n, 2, QK, L), bf16) for n in QKV_SPLIT + (DEEP,)],
            pltpu.SemaphoreType.DMA((20,)),
            [V((NT, BOTH, 2, QR, L), bf16)] * 7,
            V((TM + PAD, D), f32),
            V((3, 2, D + PAD, CW), bf16),
            V((2, CW + PAD, D), bf16),
            V((CW + PAD, D), bf16),
            V((2, 4, SLAB + PAD, 3 * D), bf16),
            V((24, 2 * SLAB + 8, L), u32),
            V((2, 4, 2 * QK + PAD, L), bf16),
            V((4, 2 * QK + PAD, L), f32),
            [V((DEEP, 2, QK, L), bf16)] * 7,
            V((7, DEEP, NCH, QR, L), bf16),
            V((8, TM + 8, L), f32),
            V((16, HALO + TM + 8, L), f32),
            V((16, HALO + TM + 8, L), f32),
            V((8, TM + 8, L), f32),
            V((2, TM, D), bf16),
            [V((DEEP, 2, QR, L), bf16)] * 7,
        ],
        compiler_params=pltpu.CompilerParams(vmem_limit_bytes=127 * 1024 * 1024, disable_bounds_checks=True),
    )(jnp.zeros((1,), jnp.int32), A_x.reshape(S, D), A_wqkv, A_wo, B_w_gate, B_w_up, B_w_down)
    return out.reshape(A_x.shape)
```

```python
import functools

import jax
import jax.numpy as jnp
import jax.experimental.pallas as pl
import jax.experimental.pallas.tpu as pltpu

S, D, F = 2048, 1024, 3584
DH, W, DIL = 32, 8, 2
L = 128
TM = 256
QR = TM // 4
NT = S // TM
QK = D // 4
CW = 4 * L
NCH = F // CW
HALO = 16
SLAB = 48
PAD = 16
LOG2E = 1.4426950408889634
f32, bf16, u32 = jnp.float32, jnp.bfloat16, jnp.uint32
part = functools.partial

A_TERMS = ((0, 1, 3), (2, 1, 3), (0,), (3,), (0, 1, 1), (2, -1, 0), (1, -1, 3))
B_TERMS = ((0, 1, 3), (0,), (1, -1, 3), (2, -1, 0), (3,), (0, 1, 1), (2, 1, 3))
C_TERMS = (((0, 1), (3, 1)), ((2, 1), (3, -1)), ((1, 1), (3, 1)), ((0, 1), (2, 1)),
           ((0, -1), (1, 1)), ((3, 1),), ((0, 1),))
C_COUNT = (4, 2, 2, 4)
OUTER = (1, 3, 4, 0, 6, 2, 5)
INNER = (1, 3, 0, 4, 6, 2, 5)
LOAD = (3, 2, 3, 3, 2, 2, 2)
FLIP = (0, 1, 0, 0, 1, 1, 1)
PLAIN, DEEP, BOTH = 4, 7, 9
PLAIN_IN_BOTH = (2, 7, 8, 3)
QKV_SPLIT = (PLAIN, PLAIN, DEEP)


def _lin(term, get):
    if len(term) == 1:
        return get(term[0])
    a, b = get(term[0]), get(term[2])
    return a + b if term[1] > 0 else a - b


def _operands(terms, split, p, get):
    flip = FLIP[p] if terms is B_TERMS else 0
    blk = [_lin(terms[p], lambda o: get(2 * (o // 2) + s // 2, 2 * (o % 2) + (s % 2 ^ flip))) for s in range(4)]
    if split == PLAIN:
        return blk
    return [_lin(t, lambda s: blk[s]) for t in terms] + ([blk[1], blk[2]] if split == BOTH else [])


def _combine(state, p, m):
    done = []
    for o, sign in C_TERMS[p]:
        if o in state:
            n, s0, acc = state[o]
            assert s0 > 0 or sign > 0
            acc = acc + m if s0 == sign else (acc - m if s0 > 0 else m - acc)
            state[o] = (n + 1, 1, acc)
            if n + 1 == C_COUNT[o]:
                done.append((o, acc))
        else:
            state[o] = (1, sign, m)
    return done


def _cat(xs, axis):
    return xs[0] if len(xs) == 1 else jnp.concatenate(xs, axis)


def _mxu(a, b):
    return jnp.dot(pltpu.bitcast(a, bf16), pltpu.bitcast(b, bf16), preferred_element_type=f32)


def _outer_product(split, p, states, lhs, rhs, sink, tick, tick_cols):
    def emit(s, m):
        s ^= FLIP[p]
        for o, val in _combine(states[s], p, m):
            sink(2 * (o // 2) + s // 2, 2 * (o % 2) + s % 2, val)

    def ticks(m):
        for b in range(tick_cols):
            for r in range(m.shape[0] // 8):
                tick(m, r, b)

    if split == DEEP:
        inner = {}
        for q in INNER:
            m = _mxu(lhs(q), rhs(q))
            for s, val in _combine(inner, q, m):
                emit(s, val)
            ticks(m)
    else:
        a = _cat([_cat([lhs(0), lhs(1)], 1), _cat([lhs(2), lhs(3)], 1)], 0)
        for j in range(2):
            m = _mxu(a, _cat([rhs(j), rhs(2 + j)], 0))
            n = m.shape[0] // 2
            emit(j, m[:n])
            emit(2 + j, m[n:])
            ticks(m)


class _Side:
    def __init__(self, jobs, span):
        self.jobs, self.span, self.n, self.done = list(jobs), span, 0, 0

    def __call__(self, m, r, b, weight=1):
        self.n += weight
        while self.done < len(self.jobs) and self.done * self.span < self.n * len(self.jobs):
            if self.jobs[self.done] is not None:
                pace, job = self.jobs[self.done]
                pace(m[r * 8:(r + 1) * 8, b * L:(b + 1) * L])
                job()
            self.done += 1

    def check(self):
        assert self.done == len(self.jobs)


def _spaced(jobs, n):
    return [j for job in jobs for j in [job] + [None] * (n - 1)]


def _merged(a, b):
    cut = lambda v, k: v[k * len(v) // 8:(k + 1) * len(v) // 8]
    return [j for k in range(8) for j in cut(a, k) + cut(b, k)]


def _run(jobs):
    for _, job in jobs:
        job()


def _rows(r, n=16):
    return pl.ds(r if isinstance(r, int) else pl.multiple_of(r, n), n)


def _words(ref):
    return ref.bitcast(u32)


def _geglu2(g, u):
    c = 0.7978845608028654
    th = jnp.tanh(g * (g * g * (c * 0.044715) + c))
    a = g * u
    return a * th + a


def _interleave_heads(cols):
    cols = list(cols)
    lane = jax.lax.broadcasted_iota(jnp.int32, cols[0].shape, 1)
    for b, s in ((1, 1), (1, 32), (1, 4), (2, 2), (2, 64), (2, 8), (4, 16)):
        m = (lane & s) != 0
        for g in range(8):
            if not g & b:
                lo, hi = cols[g], cols[g | b]
                cols[g] = jnp.where(m, pltpu.roll(hi, s, 1), lo)
                cols[g | b] = jnp.where(m, hi, pltpu.roll(lo, L - s, 1))
    return cols


def _transpose8(vs):
    vs = list(vs)
    sub = jax.lax.broadcasted_iota(jnp.int32, vs[0].shape, 0)
    for s in (1, 2, 4):
        m = (sub & s) != 0
        for g in range(8):
            if not g & s:
                lo, hi = vs[g], vs[g | s]
                vs[g] = jnp.where(m, pltpu.roll(hi, s, 0), lo)
                vs[g | s] = jnp.where(m, hi, pltpu.roll(lo, 8 - s, 0))
    return vs


def _start(copies):
    for cp in copies:
        cp.start()


def _wait(copies):
    for cp in copies:
        cp.wait()


def _kernel(zero_ref, x_hbm, wqkv_hbm, wo_hbm, wg_hbm, wu_hbm, wd_hbm, out_hbm,
            x_v, h_v, td, tq, tk, tv, to, sems, xa,
            xn, raw_gu, raw_d, raw_d6, raw_qkv, mid_qkv, raw_o, mid_o, tgu,
            ha, q_v, k_v, v_v, g_v, obuf, oa):
    zero = zero_ref[0]
    tqkv = (tq, tk, tv)
    new_states = lambda: [{} for _ in range(4)]

    def opaque(ref):
        return ref.at[pl.ds(zero, ref.shape[0])]

    def pacer(ref):
        def pace(v):
            v = pltpu.bitcast(v, u32) if ref.dtype == u32 else v.astype(ref.dtype)
            ref[(0,) * (len(ref.shape) - 2) + (_rows(ref.shape[-2] - 8 + zero, 8), pl.ds(0, L))] = v
        return pace

    def operand_jobs(src, terms, split, get, put):
        def job(p):
            for q, v in enumerate(_operands(terms, split, p, get)):
                put(p, q, v.astype(bf16))
        return [(pacer(src), part(job, p)) for p in OUTER]

    def x_copy(r):
        return pltpu.make_async_copy(x_hbm.at[_rows(r * TM, TM)], x_v.at[_rows(r * TM, TM)], sems.at[r])

    def gu0_copies(o):
        rows, cols = pl.ds((o // 2) * 2 * QK, 2 * QK), pl.ds((o % 2) * 2 * L, 2 * L)
        return [pltpu.make_async_copy(w.at[rows, cols], raw_gu.at[0, t, rows, cols], sems.at[8 + o])
                for t, w in enumerate((wg_hbm, wu_hbm))]

    def gu_copies(c):
        return [pltpu.make_async_copy(w.at[:, _rows(c * CW, CW)], raw_gu.at[c % 3, t, pl.ds(0, D)], sems.at[12 + c % 3])
                for t, w in enumerate((wg_hbm, wu_hbm))]

    def side_copies(it):
        slot, unit = it & 1, jnp.minimum(it, 3)
        sem = sems.at[15 + slot]
        r0 = pl.multiple_of(jnp.minimum(it * SLAB, QK - SLAB), 16)
        return ([pltpu.make_async_copy(wd_hbm.at[_rows(it * CW, CW)], raw_d.at[slot, pl.ds(0, CW)], sem)]
                + [pltpu.make_async_copy(wqkv_hbm.at[pl.ds(i * QK + r0, SLAB)], raw_qkv.at[slot, i, pl.ds(0, SLAB)], sem)
                   for i in range(4)]
                + [pltpu.make_async_copy(wo_hbm.at[_rows((unit >> 1) * 2 * QK, 2 * QK), _rows((2 * j + (unit & 1)) * L, L)],
                                         raw_o.at[slot, j, pl.ds(0, 2 * QK)], sem) for j in range(4)])

    def d6_copy():
        return pltpu.make_async_copy(wd_hbm.at[pl.ds((NCH - 1) * CW, CW)], raw_d6.at[pl.ds(0, CW)], sems.at[17])

    _start([x_copy(0), x_copy(1)] + [cp for o in (0, 2, 3, 1) for cp in gu0_copies(o)]
           + [x_copy(r) for r in range(2, NT)] + gu_copies(1) + gu_copies(2) + side_copies(0) + [d6_copy()])

    def norm_jobs(r):
        mean, rstd = {}, {}
        load = lambda u, z: x_v[_rows(r * TM + u * 16 + z), :].astype(f32)

        def centre(u):
            mean[u] = jnp.mean(load(u, 0), axis=-1, keepdims=True)

        def spread(u):
            xc = load(u, zero) - mean[u]
            rstd[u] = jax.lax.rsqrt(jnp.mean(xc * xc, axis=-1, keepdims=True) + 1e-5)

        def scale(u):
            xn[_rows(u * 16), :] = (load(u, 2 * zero) - mean[u]) * rstd[u]

        n = TM // 16
        return [(pacer(x_v), part(fn, u - 3 * k)) for u in range(n + 6)
                for k, fn in enumerate((centre, spread, scale)) if 0 <= u - 3 * k < n]

    def xa_jobs(r):
        def one(u, cg):
            def put(p, q, v):
                xa[p][r, q, cg, _rows(u * 16), :] = v
            get = lambda i, j: xn[_rows(i * QR + u * 16 + zero), pl.ds((2 * j + cg) * L, L)]
            return operand_jobs(xn, A_TERMS, BOTH, get, put)
        return [one(u, cg) for u in range(QR // 16) for cg in range(2)]

    def gu_jobs(slot, n):
        def one(u, t):
            def put(p, q, v):
                tgu[p][q, t, _rows(u * 16), :] = v
            get = lambda i, j: raw_gu[slot, t, _rows(i * QK + u * 16), pl.ds(j * L, L)].astype(f32)
            return operand_jobs(raw_gu, B_TERMS, DEEP, get, put)[n]
        return [one(u, t) for u in range(QK // 16) for t in range(2)]

    def wd_jobs(buf, lead, r_src, r_dst, cg):
        def put(p, q, v):
            td[p, q, cg, _rows(r_dst), :] = v
        get = lambda i, j: buf[lead + (_rows(i * L + r_src), pl.ds((2 * j + cg) * L, L))].astype(f32)
        return operand_jobs(buf, B_TERMS, DEEP, get, put)

    def qkv_permute(slot, t, u, i):
        cols = [pltpu.bitcast(raw_qkv[slot, i, _rows(u * 16), pl.ds(t * D + g * L, L)], u32) for g in range(8)]
        for g, c in enumerate(_interleave_heads(cols)):
            mid_qkv[t * 8 + g, _rows((i * SLAB + u * 16) // 2, 8), :] = c

    def qkv_jobs(r0, t, u, cg):
        def put(p, q, v):
            tqkv[t][p, q, cg, _rows(r0 + u * 16), :] = v
        get = lambda i, j: pltpu.bitcast(
            opaque(mid_qkv)[t * 8 + 2 * j + cg, _rows((i * SLAB + u * 16) // 2, 8), :], bf16).astype(f32)
        return operand_jobs(mid_qkv, B_TERMS, QKV_SPLIT[t], get, put)

    def wo_permute(slot, j, i, h1):
        old = [raw_o[slot, j, _rows((s % 4) * L + (2 * h1 + s // 4) * DH + (i // 2) * 16), :].astype(f32)
               [(i % 2) * 8:(i % 2 + 1) * 8] for s in range(8)]
        for a, v in enumerate(_transpose8(old)):
            mid_o[j, _rows(i * L + a * 16 + h1 * 8, 8), :] = v

    def wo_jobs(unit, a):
        def put(p, q, v):
            to[p, q, unit & 1, _rows(a * 32 + (unit >> 1) * 16), :] = v
        return operand_jobs(mid_o, B_TERMS, DEEP, lambda i, j: opaque(mid_o)[j ^ 2, _rows(i * L + a * 16), :], put)

    def gu_product(c, states, n, tiles, tick):
        p = OUTER[n]

        def sink(i, j, gu):
            h = _geglu2(gu[:, :L], gu[:, L:]).astype(bf16)
            for b, r in enumerate(tiles):
                h_v[c, j, _rows(r * TM + i * QR, QR), :] = h[b * QR:(b + 1) * QR]

        _outer_product(DEEP, p, states,
                       lambda q: _cat([_cat([_words(xa[p])[r + zero, q, cg] for cg in range(2)], 1) for r in tiles], 0),
                       lambda q: _cat([opaque(_words(tgu[p]))[q, t] for t in range(2)], 1), sink, tick, 1)

    @pl.loop(0, 2)
    def _(r):
        x_copy(r).wait()
        _run(norm_jobs(r) + [job for piece in xa_jobs(r) for job in piece])

    first_states = [new_states(), new_states()]

    def first(n, tiles, jobs):
        side = _Side(jobs, 56 * len(tiles) - 24)
        for r in tiles:
            gu_product(0, first_states[r], n, [r], side)
        side.check()

    g0 = part(gu_jobs, 0)
    _wait(gu0_copies(0))
    _run(g0(0))
    first(0, [0], [])
    _wait(gu0_copies(2))
    first(0, [1], g0(1))
    first(1, [0], [])
    _wait(gu0_copies(3))
    first(1, [1], g0(2))
    first(2, [0, 1], g0(3) + g0(4)[:16])
    _wait(gu0_copies(1) + [x_copy(2)])
    norm2 = norm_jobs(2)
    first(3, [0, 1], _merged(g0(4)[16:] + g0(5)[:16], norm2[:16]))
    first(4, [0, 1], _merged(g0(5)[16:] + g0(6)[:8], norm2[16:24]))
    first(5, [0, 1], _merged(g0(6)[8:], norm2[24:32]))
    first(6, [0, 1], norm2[32:] + [piece[0] for piece in xa_jobs(2)])

    @pl.loop(2, NT)
    def _(r):
        nxt = jnp.minimum(r + 1, NT - 1)
        pl.when(r + 1 < NT)(x_copy(nxt).wait)
        jobs = ([piece[n] for n in range(1, 7) for piece in xa_jobs(r)]
                + norm_jobs(nxt) + [piece[0] for piece in xa_jobs(nxt)])
        side = _Side(jobs, 56 * sum(LOAD) - 16)
        states = new_states()
        for n in range(7):
            gu_product(0, states, n, [r], part(side, weight=LOAD[n]))
        side.check()

    _wait(gu_copies(1) + [d6_copy()])
    _run(gu_jobs(1, 0))

    @pl.loop(1, NCH)
    def _(c):
        it = c - 1
        slot, nxt = it & 1, jnp.minimum(c + 1, NCH - 1)
        pl.when(c + 1 < NCH)(lambda: _wait(gu_copies(nxt)))
        _wait(side_copies(it))
        for cp in side_copies(c):
            pl.when(c + 1 < NCH)(cp.start)
        for cp in gu_copies(jnp.minimum(c + 2, NCH - 1)):
            pl.when(c + 2 < NCH)(cp.start)

        r0 = jnp.minimum(it * SLAB, QK - SLAB)
        r6 = jnp.minimum(it * 32, L - 32)
        jobs = []
        for cg in range(2):
            for u in range(L // 16):
                jobs += wd_jobs(raw_d, (slot,), u * 16, it * L + u * 16, cg)
            for u in range(2):
                jobs += wd_jobs(raw_d6, (), r6 + u * 16, (NCH - 1) * L + r6 + u * 16, cg)
        slabs = [(t, u) for t in range(3) for u in range(SLAB // 16)]
        for n, (t, u, i) in enumerate((t, u, i) for t, u in slabs for i in range(4)):
            jobs.insert(4 * n, (pacer(raw_qkv), part(qkv_permute, slot, t, u, i)))
        jobs += [(pacer(raw_o), part(wo_permute, slot, j, i, h1)) for j in range(4) for i in range(4) for h1 in range(2)]
        jobs += [job for t, u in slabs for cg in range(2) for job in qkv_jobs(r0, t, u, cg)]
        jobs += [job for a in range(8) for job in wo_jobs(jnp.minimum(it, 3), a)]
        per_product = 7 * NT * QR // 8
        extra = _Side(jobs, sum(LOAD) * per_product - 300)
        states = new_states()
        for n in range(7):
            side = _Side(gu_jobs(c % 3, n + 1) if n < 6 else gu_jobs(nxt % 3, 0), per_product - 200)
            gu_product(c, states, n, range(NT), lambda *a: (side(*a), extra(*a, weight=LOAD[n])))
            side.check()
        extra.check()

    def out_copies(r):
        return [pltpu.make_async_copy(obuf.at[r & 1, pl.ds(i * QR, QR), pl.ds(j * QK, QK)],
                                      out_hbm.at[_rows(r * TM + i * QR, QR), pl.ds(j * QK, QK)], sems.at[18 + (r & 1)])
                for i in range(4) for j in range(4)]

    def project(split, lhs, rhs, sink, tick, tick_cols):
        states = new_states()
        for n, p in enumerate(OUTER):
            _outer_product(split, p, states, part(lhs, p), part(rhs, p), sink, part(tick, n), tick_cols)

    for g in range(8):
        k_v[g, pl.ds(TM, HALO), :] = jnp.zeros((HALO, L), f32)
        v_v[g, pl.ds(TM, HALO), :] = jnp.zeros((HALO, L), f32)

    @pl.loop(0, NT)
    def _(r):
        pl.when(r >= 2)(lambda: _wait(out_copies(r - 2)))
        for g in range(8):
            k_v[g, pl.ds(0, HALO), :] = k_v[g, pl.ds(TM, HALO), :]
            v_v[g, pl.ds(0, HALO), :] = v_v[g, pl.ds(TM, HALO), :]

        def h_jobs(c, u):
            def put(p, q, v):
                ha[p, q, c, _rows(u * 16), :] = v
            get = lambda i, j: h_v[c, j, _rows(r * TM + i * QR + u * 16), :].astype(f32)
            return operand_jobs(h_v, A_TERMS, DEEP, get, put)

        q_o, k_o, v_o, g_o = (opaque(ref) for ref in (q_v, k_v, v_v, g_v))
        window = lambda r0, w: pl.ds(r0 + HALO - DIL * w, 16)
        cells = [(r0, w) for r0 in range(0, TM, 16) for w in range(W)]
        held = {}

        def logits(r0, w):
            k_v[8 + w, _rows(r0), :] = functools.reduce(
                jnp.add, [q_o[g, _rows(r0), :] * k_o[g, window(r0, w), :] for g in range(8)])

        def rotate(r0, w):
            held[r0, w] = [pltpu.roll(k_o[8 + w, _rows(r0), :], s, 1) for s in (32, 64, 96)]

        def fold(r0, w):
            l = functools.reduce(jnp.add, held[r0, w], k_o[8 + w, _rows(r0), :])
            if r0 < HALO and w > 0:
                pos = r * TM + r0 + jax.lax.broadcasted_iota(jnp.int32, l.shape, 0)
                l = jnp.where(pos >= DIL * w, l, -1e9 * LOG2E)
            held[r0, w] = l

        def keep(r0, w):
            k_v[8 + w, _rows(r0), :] = held[r0, w]

        def logit_step(n):
            for fn, lag in ((rotate, 2), (fold, 7), (logits, 0), (keep, 7)):
                if 0 <= n - lag < len(cells):
                    fn(*cells[n - lag])

        def softmax(r0):
            ls = [k_o[8 + w, _rows(r0, 8), :] for w in range(W)]
            top = functools.reduce(jnp.maximum, ls)
            ps = [jnp.exp2(l - top) for l in ls]
            inv = 1.0 / functools.reduce(jnp.add, ps)
            for w in range(W):
                k_v[8 + w, _rows(r0, 8), :] = ps[w] * inv

        def mix(r0, g):
            v_v[8 + g, _rows(r0), :] = functools.reduce(
                jnp.add, [k_o[8 + w, _rows(r0), :] * v_o[g, window(r0, w), :] for w in range(W)])

        def o_jobs(u, cg):
            def put(p, q, v):
                oa[p][q, cg, _rows(u * 16), :] = v
            return operand_jobs(v_v, A_TERMS, DEEP, lambda i, j: v_o[8 + 2 * j + cg, _rows(i * QR + u * 16), :], put)

        pieces = [o_jobs(u, cg) for u in range(QR // 16) for cg in range(2)]
        attn = _Side(_spaced([(pacer(k_v), part(logit_step, n)) for n in range(len(cells) + 7)], 5)
                     + _spaced([(pacer(k_v), part(softmax, r0)) for r0 in range(0, TM, 8)], 4)
                     + _spaced([(pacer(v_v), part(mix, r0, g)) for r0 in range(0, TM, 16) for g in range(8)], 2)
                     + _spaced([piece[n] for n in range(7) for piece in pieces], 2),
                     5 * 392 + 112 * (sum(LOAD) + 14) - 256)
        side = _Side([job for c in range(NCH) for u in range(QR // 16) for job in h_jobs(c, u)],
                     8 * 896 + 3 * 392 - 400)

        for t, dst, off in ((1, k_v, HALO), (0, q_v, 0), (2, v_v, HALO)):
            def sink(i, j, val):
                if t == 0:
                    val = val * (DH ** -0.5 * LOG2E)
                for cg in range(2):
                    piece = val[:, cg * L:(cg + 1) * L]
                    dst[2 * j + cg, pl.ds(off + i * QR, QR), :] = piece
                    if t == 2 and i == 0:
                        dst[2 * j + cg, pl.ds(0, HALO), :] = jnp.where(
                            r == 0, jnp.broadcast_to(piece[0:1], (HALO, L)), dst[2 * j + cg, pl.ds(0, HALO), :])

            deep = QKV_SPLIT[t] == DEEP
            project(QKV_SPLIT[t],
                    lambda p, q: _cat([_words(xa[p])[r, q if deep else PLAIN_IN_BOTH[q], cg] for cg in range(2)], 1),
                    lambda p, q: _cat([_words(tqkv[t])[p, q, cg] for cg in range(2)], 1), sink,
                    (lambda n, *a: side(*a, weight=8)) if t < 2 else (lambda n, *a: (side(*a, weight=3), attn(*a, weight=5))),
                    1 if deep else 2)
        side.check()

        def gate_sink(i, j, val):
            half = val * 0.25
            gate = half * jnp.tanh(half) + half
            for cg in range(2):
                g_v[2 * j + cg, pl.ds(i * QR, QR), :] = gate[:, cg * L:(cg + 1) * L]

        project(DEEP, lambda p, q: _cat([opaque(_words(ha))[p, q, c] for c in range(NCH)], 1),
                lambda p, q: _cat([_words(td)[p, q, cg] for cg in range(2)], 1), gate_sink,
                lambda n, *a: attn(*a, weight=LOAD[n] + 2), 2)
        attn.check()

        copies = out_copies(r)

        def out_sink(i, j, val):
            j ^= 2
            cols = pl.ds(j * QK, QK)
            gate = _cat([g_o[2 * j + cg, pl.ds(i * QR, QR), :] for cg in range(2)], 1)
            res = x_v[_rows(r * TM + i * QR, QR), cols].astype(f32) + val * gate
            obuf[r & 1, pl.ds(i * QR, QR), cols] = res.astype(obuf.dtype)
            copies[4 * i + j].start()

        project(DEEP, lambda p, q: _cat([opaque(_words(oa[p]))[q, cg] for cg in range(2)], 1),
                lambda p, q: _cat([_words(to)[p, q, cg] for cg in range(2)], 1), out_sink, lambda *a: None, 0)

    _wait(out_copies(NT - 2) + out_copies(NT - 1))


@jax.jit
def pallas_recurrent_scan__sliding_local_dilated__geglu_ffn__prompt_kernel(
    A_x: jax.Array,
    A_wqkv: jax.Array,
    A_wo: jax.Array,
    B_x: jax.Array,
    B_w_gate: jax.Array,
    B_w_up: jax.Array,
    B_w_down: jax.Array,
):
    del B_x
    hbm = pl.BlockSpec(memory_space=pl.ANY)
    V = pltpu.VMEM
    out = pl.pallas_call(
        _kernel,
        in_specs=[pl.BlockSpec(memory_space=pltpu.SMEM)] + [hbm] * 6,
        out_specs=hbm,
        out_shape=jax.ShapeDtypeStruct((S, D), bf16),
        scratch_shapes=[
            V((S + PAD, D), bf16),
            V((NCH, 4, S + PAD, L), bf16),
            V((7, DEEP, 2, F // 4, L), bf16),
            *[V((7, n, 2, QK, L), bf16) for n in QKV_SPLIT + (DEEP,)],
            pltpu.SemaphoreType.DMA((20,)),
            [V((NT, BOTH, 2, QR, L), bf16)] * 7,
            V((TM + PAD, D), f32),
            V((3, 2, D + PAD, CW), bf16),
            V((2, CW + PAD, D), bf16),
            V((CW + PAD, D), bf16),
            V((2, 4, SLAB + PAD, 3 * D), bf16),
            V((24, 2 * SLAB + 8, L), u32),
            V((2, 4, 2 * QK + PAD, L), bf16),
            V((4, 2 * QK + PAD, L), f32),
            [V((DEEP, 2, QK, L), bf16)] * 7,
            V((7, DEEP, NCH, QR, L), bf16),
            V((8, TM + 8, L), f32),
            V((16, HALO + TM + 8, L), f32),
            V((16, HALO + TM + 8, L), f32),
            V((8, TM + 8, L), f32),
            V((2, TM, D), bf16),
            [V((DEEP, 2, QR, L), bf16)] * 7,
        ],
        compiler_params=pltpu.CompilerParams(vmem_limit_bytes=127 * 1024 * 1024, disable_bounds_checks=True),
    )(jnp.zeros((1,), jnp.int32), A_x.reshape(S, D), A_wqkv, A_wo, B_w_gate, B_w_up, B_w_down)
    return out.reshape(A_x.shape)
```
